```python
import os as _os
_os.environ.setdefault("JAX_PLATFORMS", "cpu")
import jax
import jax.numpy as jnp

def _softmax(x, axis=-1):
    return jax.nn.softmax(x, axis=axis)
def _gelu(x):
    return jax.nn.gelu(x, approximate=True)
def _silu(x):
    return jax.nn.silu(x)
def _sigmoid(x):
    return jax.nn.sigmoid(x)
def _layernorm(x, axis=-1, eps=1e-5):
    m = jnp.mean(x, axis=axis, keepdims=True)
    v = jnp.var(x, axis=axis, keepdims=True)
    return (x - m) / jnp.sqrt(v + eps)
def _scatter_add(tgt, idx, src, axis=0):
    return tgt.at[idx].add(src)
def _segment_sum(src, seg, n):
    return jax.ops.segment_sum(src, seg, n)
class _Rng:
    def __init__(self, key):
        self._k = key
    def _next(self):
        self._k, sub = jax.random.split(self._k)
        return sub
    def normal(self, shape):
        return jax.random.normal(self._next(), shape, dtype=jnp.bfloat16)
    def randint(self, lo, hi, shape):
        return jax.random.randint(self._next(), shape, lo, hi, dtype=jnp.int32)
    def uniform(self, shape, lo=0.0, hi=1.0):
        return jax.random.uniform(self._next(), shape, jnp.bfloat16, lo, hi)
    def permutation(self, n):
        return jax.random.permutation(self._next(), n)


kernel_name = 'sequential_preLN__sliding_block__glu_gated_swiglu__prompt'

def setup_inputs():
    _rng = _Rng(jax.random.key(int.from_bytes(__import__("os").urandom(4), "little")))
    _w = (lambda a: (lambda t: t.astype(jnp.bfloat16) if jnp.issubdtype(t.dtype, jnp.floating) else t)(jnp.asarray(a)))
    def _A_setup():
        B, S, D = 1, 2048, 640
        return {
            "x": _w((lambda *s: _rng.normal(s) * 0.05)(B, S, D)),
            "wqkv": _w((lambda *s: _rng.normal(s) * 0.05)(D, 3 * D)),
            "wo": _w((lambda *s: _rng.normal(s) * 0.05)(D, D)),
        }
    _A_in = _A_setup()

    def _B_setup():
        B, S, D, F = 1, 2048, 640, 1728
        return {
            "x": _w((lambda *s: _rng.normal(s) * 0.05)(B, S, D)),
            "w1": _w((lambda *s: _rng.normal(s) * 0.1)(D, F) * (2.0 / D) ** 0.5),
            "w3": _w((lambda *s: _rng.normal(s) * 0.1)(D, F) * (2.0 / D) ** 0.5),
            "w2": _w((lambda *s: _rng.normal(s) * 0.1)(F, D) * (2.0 / F) ** 0.5),
        }
    _B_in = _B_setup()

    return {
        "A_x": _A_in["x"],
        "A_wqkv": _A_in["wqkv"],
        "A_wo": _A_in["wo"],
        "B_x": _B_in["x"],
        "B_w1": _B_in["w1"],
        "B_w3": _B_in["w3"],
        "B_w2": _B_in["w2"],
    }

def reference(A_x, A_wqkv, A_wo, B_x, B_w1, B_w3, B_w2):
    def _A_ref(x, wqkv, wo):
        B, S, D = x.shape
        H = 32; Dh = D // H; W = 256
        qkv = (lambda x, *d: x.transpose(*d))((x @ wqkv).reshape(B, S, 3, H, Dh), 2, 0, 3, 1, 4)
        q, k, v = qkv[0], qkv[1], qkv[2]
        scores = jnp.einsum("bhqd,bhkd->bhqk", q, k) * (Dh ** -0.5)
        idx = jnp.arange(S)
        mask = (idx[:, None] - idx[None, :] >= 0) & (idx[:, None] - idx[None, :] < W)
        scores = jnp.where(mask[None, None], scores, -1e9)
        p = _softmax(scores, axis=-1)
        o = jnp.einsum("bhqk,bhkd->bhqd", p, v)
        return (lambda x, *d: x.transpose(*d))(o, 0, 2, 1, 3).reshape(B, S, D) @ wo

    def _B_ref(x, w1, w3, w2):
        gate = jnp.einsum("bsd,df->bsf", x, w1)
        up = jnp.einsum("bsd,df->bsf", x, w3)
        h = _silu(gate) * up
        out = jnp.einsum("bsf,fd->bsd", h, w2)
        return out

    x = A_x
    h = x + _A_ref(_layernorm(x, axis=-1), A_wqkv, A_wo)
    h2 = h + _B_ref(_layernorm(h, axis=-1), B_w1, B_w3, B_w2)
    return h2
```

```python
import functools
import math
import jax
import jax.numpy as jnp
from jax import lax
import jax.experimental.pallas as pl
import jax.experimental.pallas.tpu as pltpu

S, D, H, DH, WIN, F = 2048, 640, 32, 20, 256, 1728
T = 256
QB = 128
NG = 8
EPS = 1e-5
NEG = -1e30
QSCALE = (DH ** -0.5) * math.log2(math.e)
FCH = 256
ONE2 = 0x3F803F80

def _ln(x):
    m = jnp.mean(x, axis=-1, keepdims=True)
    xc = x - m
    v = jnp.mean(xc * xc, axis=-1, keepdims=True)
    return xc * lax.rsqrt(v + EPS)

def _u32(x):
    return pltpu.bitcast(x, jnp.uint32)

def _b16(x):
    return pltpu.bitcast(x, jnp.bfloat16)

def _group_tile(a_u32, g, lane):
    lo = 80 * g
    ta = lo // 128
    off = lo % 128
    A = a_u32[:, ta * 128:(ta + 1) * 128]
    if off + 80 <= 128:
        return jnp.where((lane >= off) & (lane < off + 80), A, jnp.uint32(0))
    B = a_u32[:, (ta + 1) * 128:(ta + 2) * 128]
    rem = off + 80 - 128
    return jnp.where(lane >= off, A, jnp.where(lane < rem, B, jnp.uint32(0)))

def kernel(x_ref, wqkv_hbm, wo_hbm, w1_hbm, w3_hbm, w2_hbm, o_ref,
           wqkv_v, wo_v, w1_v, w3_v, w2_v, wvt_v, kext, vt, qext, ot, sems):
    step = pl.program_id(0)
    copies = [
        pltpu.make_async_copy(wqkv_hbm, wqkv_v, sems.at[0]),
        pltpu.make_async_copy(wo_hbm, wo_v, sems.at[1]),
        pltpu.make_async_copy(w1_hbm, w1_v, sems.at[2]),
        pltpu.make_async_copy(w3_hbm, w3_v, sems.at[3]),
        pltpu.make_async_copy(w2_hbm, w2_v, sems.at[4]),
    ]

    @pl.when(step == 0)
    def _():
        for c in copies:
            c.start()
        lane = lax.broadcasted_iota(jnp.int32, (WIN, 128), 1)
        for g in range(NG):
            bl = (80 * g + 80) % 128
            kext[0:WIN, g * 128:(g + 1) * 128] = jnp.where(lane == bl, NEG, 0.0).astype(jnp.bfloat16)
        vt[0:2] = jnp.zeros((2, D, 128), jnp.bfloat16)
        copies[0].wait()
        wv = wqkv_v[:, 2 * D:3 * D].astype(jnp.float32)
        wvt_v[...] = wv.T.astype(jnp.bfloat16)

    x = x_ref[0].astype(jnp.float32)
    xn = _ln(x).astype(jnp.bfloat16)
    q = jnp.dot(xn, wqkv_v[:, 0:D], preferred_element_type=jnp.float32)
    k = jnp.dot(xn, wqkv_v[:, D:2 * D], preferred_element_type=jnp.float32)
    vT = lax.dot_general(wvt_v[...], xn, (((1,), (1,)), ((), ())), preferred_element_type=jnp.float32)
    qu = _u32((q * QSCALE).astype(jnp.bfloat16))
    ku = _u32(k.astype(jnp.bfloat16))
    lane_h = lax.broadcasted_iota(jnp.int32, (T // 2, 128), 1)
    row0 = pl.multiple_of(step * T + WIN, T)
    for g in range(NG):
        qext[:, g * 128:(g + 1) * 128] = _b16(_group_tile(qu, g, lane_h))
        kext[pl.ds(row0, T), g * 128:(g + 1) * 128] = _b16(_group_tile(ku, g, lane_h))
    vTb = vT.astype(jnp.bfloat16)
    nb = T // QB
    for b in range(nb):
        vt[step * nb + 2 + b] = vTb[:, b * 128:(b + 1) * 128]

    lane16 = lax.broadcasted_iota(jnp.int32, (16, 128), 1)
    lane32 = lax.broadcasted_iota(jnp.int32, (32, 128), 1)
    row32 = lax.broadcasted_iota(jnp.int32, (32, 128), 0)
    tri = row32 > (lane32 % 32)
    quarter16 = lane16 // 32
    m_even = (quarter16 % 2) == 0
    m_lo = quarter16 < 2
    m_mid = (quarter16 == 1) | (quarter16 == 2)
    sub8 = lax.broadcasted_iota(jnp.int32, (8, 128), 0)
    sub16u = lax.broadcasted_iota(jnp.int32, (16, 384), 0)

    def sel(mask, a, b):
        if a is None and b is None:
            return None
        z = jnp.zeros((16, 128), jnp.uint32)
        return jnp.where(mask, z if a is None else a, z if b is None else b)

    for b in range(nb):
        kbase = step * T + b * QB
        vblk = step * nb + b
        for g in range(NG):
            u = (lane16 - 80 * g) % 128
            biasc = jnp.where(u == 80, jnp.uint32(ONE2), jnp.uint32(0))
            hm = [(u >= 20 * hh) & (u < 20 * hh + 20) for hh in range(4)]
            A = []
            for j in range(4):
                q32 = _u32(qext[b * QB + 32 * j: b * QB + 32 * j + 32, g * 128:(g + 1) * 128])
                w = jnp.concatenate([jnp.where(hm[(p - j) % 4], q32, biasc) for p in range(4)], axis=0)
                kj = kext[pl.ds(pl.multiple_of(kbase + 32 * j, 32), 288), g * 128:(g + 1) * 128]
                s = lax.dot_general(kj, _b16(w), (((1,), (1,)), ((), ())), preferred_element_type=jnp.float32)
                sf = jnp.where(tri, s[0:32], s[256:288])
                sm = s[32:256]
                m = jnp.maximum(jnp.max(sm, axis=0, keepdims=True), jnp.max(sf, axis=0, keepdims=True))
                pf = jnp.exp2(sf - m)
                pm = jnp.exp2(sm - m)
                p_first = jnp.where(tri, pf, 0.0).astype(jnp.bfloat16)
                p_last = jnp.where(tri, 0.0, pf).astype(jnp.bfloat16)
                pmu = _u32(pm.astype(jnp.bfloat16))
                blocks = [_u32(p_first)] + [pmu[16 * i:16 * i + 16] for i in range(7)] + [_u32(p_last)]
                A.append(blocks)
            B = [[], [], [], []]
            for t in range(12):
                a = [A[j][t - j] if 0 <= t - j <= 8 else None for j in range(4)]
                d0 = sel(m_even, a[0], a[1]); d1 = sel(m_even, a[1], a[0])
                d2 = sel(m_even, a[2], a[3]); d3 = sel(m_even, a[3], a[2])
                B[0].append(sel(m_lo, d0, d2)); B[2].append(sel(m_lo, d2, d0))
                B[1].append(sel(m_mid, d1, d3)); B[3].append(sel(m_mid, d3, d1))
            outs = []
            for hh in range(4):
                pT = _b16(jnp.concatenate(B[hh], axis=0))
                r0 = 80 * g + 16 * hh
                vw = jnp.concatenate([vt[vblk + i, r0:r0 + 32, :] for i in range(3)], axis=1)
                vwu = _u32(vw)
                if hh < 2:
                    vwu = jnp.where(sub16u >= 12, jnp.uint32(ONE2), vwu)
                else:
                    vwu = jnp.where(sub16u < 4, jnp.uint32(ONE2), vwu)
                o = jnp.dot(_b16(vwu), pT, preferred_element_type=jnp.float32)
                if hh < 2:
                    den = o[24:32]; val = o[0:24]
                else:
                    den = o[0:8]; val = o[8:32]
                inv = 1.0 / den
                val = val * jnp.concatenate([inv, inv, inv], axis=0)
                if hh:
                    val = pltpu.roll(val, 128 - 32 * hh, 1)
                outs.append(val)
            v2 = jnp.where(sub8 < 4, outs[0][16:24], outs[1][0:8])
            v7 = jnp.where(sub8 < 4, outs[2][16:24], outs[3][0:8])
            og = jnp.concatenate([outs[0][0:16], v2, outs[1][8:24], outs[2][0:16], v7, outs[3][8:24]], axis=0)
            ot[80 * g:80 * g + 80, b * QB:(b + 1) * QB] = og

    @pl.when(step == 0)
    def _():
        copies[1].wait()

    o_nat = ot[...].T.astype(jnp.bfloat16)
    h = x + jnp.dot(o_nat, wo_v[...], preferred_element_type=jnp.float32)
    hn = _ln(h).astype(jnp.bfloat16)

    @pl.when(step == 0)
    def _():
        copies[2].wait()
        copies[3].wait()
        copies[4].wait()

    acc = h
    c0 = 0
    while c0 < F:
        c1 = min(c0 + FCH, F)
        gate = jnp.dot(hn, w1_v[:, c0:c1], preferred_element_type=jnp.float32)
        up = jnp.dot(hn, w3_v[:, c0:c1], preferred_element_type=jnp.float32)
        act = (gate * jax.nn.sigmoid(gate) * up).astype(jnp.bfloat16)
        acc = acc + jnp.dot(act, w2_v[c0:c1, :], preferred_element_type=jnp.float32)
        c0 = c1
    o_ref[0] = acc.astype(o_ref.dtype)


@jax.jit
def pallas_sequential_preLN__sliding_block__glu_gated_swiglu__prompt_kernel(A_x, A_wqkv, A_wo, B_x, B_w1, B_w3, B_w2):
    bf = jnp.bfloat16
    any_spec = pl.BlockSpec(memory_space=pl.ANY)
    return pl.pallas_call(
        kernel,
        grid=(S // T,),
        in_specs=[pl.BlockSpec((1, T, D), lambda i: (0, i, 0))] + [any_spec] * 5,
        out_specs=pl.BlockSpec((1, T, D), lambda i: (0, i, 0)),
        out_shape=jax.ShapeDtypeStruct((1, S, D), bf),
        scratch_shapes=[
            pltpu.VMEM((D, 3 * D), bf), pltpu.VMEM((D, D), bf), pltpu.VMEM((D, F), bf),
            pltpu.VMEM((D, F), bf), pltpu.VMEM((F, D), bf), pltpu.VMEM((D, D), bf),
            pltpu.VMEM((S + WIN, NG * 128), bf), pltpu.VMEM((S // 128 + 2, D, 128), bf),
            pltpu.VMEM((T, NG * 128), bf), pltpu.VMEM((D, T), jnp.float32),
            pltpu.SemaphoreType.DMA((5,)),
        ],
        compiler_params=pltpu.CompilerParams(dimension_semantics=("arbitrary",),
                                             vmem_limit_bytes=100 * 1024 * 1024),
    )(A_x, A_wqkv, A_wo, B_w1, B_w3, B_w2)
```

```python
import contextlib
import functools
import math
import os
import jax
import jax.numpy as jnp
from jax import lax
import jax.experimental.pallas as pl
import jax.experimental.pallas.tpu as pltpu

VAR = os.environ.get('VAR', '0F1P2F3,0F1FP2F3')
VAR0 = os.environ.get('VAR0', 'abPF')
VAR1 = os.environ.get('VAR1', 'aFPbF')
VAR7 = os.environ.get('VAR7', 'aFbFPF')
NFIRST = int(os.environ.get('NFIRST', '5'))
CHAIN = int(os.environ.get('CHAIN', '3'))
CHAIN0 = int(os.environ.get('CHAIN0', '3'))
KA = int(os.environ.get('KA', '2'))
KEEP1 = int(os.environ.get('KEEP1', '3'))
SCOPES = int(os.environ.get('SCOPES', '0'))
ONLY = os.environ.get('ONLY', '')

S, D, H, DH, WIN, F = 2048, 640, 32, 20, 256, 1728
T = 256
QB = 128
NB = T // QB
NG = 8
NSTEP = S // T
EPS = 1e-5
QSCALE = (DH ** -0.5) * math.log2(math.e)
FMAIN = 1664
FA = 128 * NFIRST
ONE2 = 0x3F803F80
NEGBIG = -1e30
NT = (((1,), (1,)), ((), ()))
f32 = jnp.float32
bf16 = jnp.bfloat16
u32 = jnp.uint32
NW = 10


def scope(name):
    return jax.named_scope(name) if SCOPES else contextlib.nullcontext()


def _ln(x):
    m = jnp.mean(x, axis=-1, keepdims=True)
    xc = x - m
    v = jnp.mean(xc * xc, axis=-1, keepdims=True)
    return xc * lax.rsqrt(v + EPS)


def _u32(x):
    return pltpu.bitcast(x, u32)


def _b16(x):
    return pltpu.bitcast(x, bf16)


def _pack32(x):
    n = x.shape[0] // 32
    return jnp.concatenate(
        [pltpu.pack_elementwise([x[32 * i:32 * i + 16], x[32 * i + 16:32 * i + 32]], packed_dtype=bf16).astype(u32)
         for i in range(n)], axis=0)


def _group_tile(tiles, g, lane):
    lo = 80 * g
    ta = lo // 128
    off = lo % 128
    if off + 80 <= 128:
        return tiles[ta]
    return jnp.where(lane >= off, tiles[ta], tiles[ta + 1])


def _silu_mul(g, u):
    hg = 0.5 * g
    return (hg * (1.0 + jnp.tanh(hg))) * u


def _ds(start, n, align):
    if isinstance(start, int):
        return pl.ds(start, n)
    return pl.ds(pl.multiple_of(start, align), n)


def kernel(x_hbm, wqkv_hbm, wo_hbm, w1_hbm, w3_hbm, w2_hbm, o_hbm,
           x_v, o_v, wqkv_v, wo_v, w1_v, w3_v, w2_v, wvt_v, kext, vt, qext, h_scr, hn_scr, act_scr,
           wsem, osem):
    P = functools.partial

    def wcopy(src, dst, k):
        return pltpu.make_async_copy(src, dst, wsem.at[k])

    ks = D + 128 * KA
    cp_ka = wcopy(wqkv_hbm.at[:, D:ks], wqkv_v.at[:, D:ks], 0)
    cp_kb = wcopy(wqkv_hbm.at[:, ks:2 * D], wqkv_v.at[:, ks:2 * D], 9)
    cp_q = wcopy(wqkv_hbm.at[:, 0:D], wqkv_v.at[:, 0:D], 1)
    cp_v = wcopy(wqkv_hbm.at[:, 2 * D:3 * D], wqkv_v.at[:, 2 * D:3 * D], 2)
    cp_o = wcopy(wo_hbm, wo_v, 3)
    cp_1a = wcopy(w1_hbm.at[0:FA, :], w1_v.at[0:FA, :], 4)
    cp_3a = wcopy(w3_hbm.at[0:FA, :], w3_v.at[0:FA, :], 5)
    cp_1b = wcopy(w1_hbm.at[FA:F, :], w1_v.at[FA:F, :], 6)
    cp_3b = wcopy(w3_hbm.at[FA:F, :], w3_v.at[FA:F, :], 7)
    cp_2 = wcopy(w2_hbm, w2_v, 8)

    def xcopy(i):
        r = _ds(i * T, T, T)
        return pltpu.make_async_copy(x_hbm.at[0, r, :], x_v.at[r, :], wsem.at[NW + i])

    def ocopy(qb, nqb):
        r = _ds(qb * QB, nqb * QB, QB)
        return pltpu.make_async_copy(o_v.at[r, :], o_hbm.at[0, r, :], osem.at[qb])

    def ocopy_col(qb, nqb, n):
        r = _ds(qb * QB, nqb * QB, QB)
        return pltpu.make_async_copy(o_v.at[r, 128 * n:128 * n + 128], o_hbm.at[0, r, 128 * n:128 * n + 128],
                                     osem.at[S // QB + n])

    def ffn_first(get_hn, lb, nqb):
        st = {}
        pr = _ds(lb * 64, nqb * 64, 64)

        def gpart(c):
            st['g'] = lax.dot_general(_b16(get_hn()), w1_v[128 * c:128 * c + 128, :], NT, preferred_element_type=f32)

        def upart(c):
            u = lax.dot_general(_b16(get_hn()), w3_v[128 * c:128 * c + 128, :], NT, preferred_element_type=f32)
            act_scr[pr, 128 * c:128 * c + 128] = _u32(_silu_mul(st['g'], u).astype(bf16))

        ps = []
        for c in range(NFIRST):
            ps += [P(gpart, c), P(upart, c)]
        return ps

    def ffn_rest(qb, lb, nqb, colcopy):
        acts = []
        st = {}
        pr = _ds(lb * 64, nqb * 64, 64)
        fr = _ds(lb * QB, nqb * QB, QB)
        orow = _ds(qb * QB, nqb * QB, QB)

        def gpart(c):
            st['g'] = lax.dot_general(_b16(hn_scr[pr, :]), w1_v[128 * c:128 * c + 128, :], NT,
                                      preferred_element_type=f32)

        def upart(c):
            u = lax.dot_general(_b16(hn_scr[pr, :]), w3_v[128 * c:128 * c + 128, :], NT, preferred_element_type=f32)
            acts.append(_silu_mul(st['g'], u).astype(bf16))

        def tail():
            w = jnp.concatenate([w1_v[FMAIN:F, :], w3_v[FMAIN:F, :]], axis=0)
            r = lax.dot_general(_b16(hn_scr[pr, :]), w, NT, preferred_element_type=f32)
            acts.append(_silu_mul(r, pltpu.roll(r, 64, 1))[:, 0:64].astype(bf16))

        def w2a(n):
            a = jnp.concatenate([_b16(act_scr[pr, :])] + acts[0:7 - NFIRST], axis=1)
            hp = st['h', n] if ('h', n) in st else h_scr[fr, 128 * n:128 * n + 128]
            st['h', n] = None
            st['o'] = hp + jnp.dot(a, w2_v[0:896, 128 * n:128 * n + 128], preferred_element_type=f32)

        def w2b(n):
            a = jnp.concatenate(acts[7 - NFIRST:], axis=1)
            r = st['o'] + jnp.dot(a, w2_v[896:F, 128 * n:128 * n + 128], preferred_element_type=f32)
            o_v[orow, 128 * n:128 * n + 128] = r.astype(bf16)
            if colcopy:
                ocopy_col(qb, nqb, n).start()
            elif n == 4:
                ocopy(qb, nqb).start()

        def preload():
            for n in range(5):
                if ('h', n) not in st:
                    st['h', n] = h_scr[fr, 128 * n:128 * n + 128]

        gu = []
        for c in range(NFIRST, 13):
            gu += [P(gpart, c), P(upart, c)]
        gu.append(tail)
        w2 = []
        for n in range(5):
            w2 += [P(w2a, n), P(w2b, n)]
        return gu, w2, preload

    def qkv_pieces(i):
        st = {'k': [], 'q': [], 'v': []}

        def ln1():
            if 'xn' not in st:
                xnf = _ln(x_v[_ds(i * T, T, T), :].astype(f32))
                st['xn'] = xnf.astype(bf16)
                st['xni'] = _b16(_pack32(xnf))

        def kpart(n):
            ln1()
            k = jnp.dot(st['xn'], wqkv_v[:, D + 128 * n:D + 128 * n + 128], preferred_element_type=f32)
            st['k'].append(_u32(k.astype(bf16)))

        def qpart(n):
            q = jnp.dot(st['xn'], wqkv_v[:, 128 * n:128 * n + 128], preferred_element_type=f32)
            st['q'].append(_u32((q * QSCALE).astype(bf16)))

        def vpart(n):
            v = lax.dot_general(_b16(wvt_v[64 * n:64 * n + 64, :]), st['xni'], NT, preferred_element_type=f32)
            st['v'].append(_u32(v.astype(bf16)))

        def store():
            lane = lax.broadcasted_iota(jnp.int32, (T // 2, 128), 1)
            for g in range(NG):
                qext[g] = _group_tile(st['q'], g, lane)
                kext[g, _ds(i * (T // 2), T // 2, T // 2), :] = _group_tile(st['k'], g, lane)
            for n in range(5):
                for b in range(NB):
                    vt[i * NB + b, 64 * n:64 * n + 64, :] = st['v'][n][:, b * 128:(b + 1) * 128]

        return ([P(kpart, n) for n in range(5)], [P(qpart, n) for n in range(5)], [P(vpart, n) for n in range(5)],
                store, ln1)

    def run_fill(pieces, n, keep):
        for _ in range(n):
            if len(pieces) > keep:
                pieces.pop(0)()

    def attention(qb, lb, nqb, pieces, patterns, keep, chain):
        patterns = patterns.split(',')
        lane16 = lax.broadcasted_iota(jnp.int32, (16, 128), 1)
        lane32 = lax.broadcasted_iota(jnp.int32, (32, 128), 1)
        row32 = lax.broadcasted_iota(jnp.int32, (32, 128), 0)
        tri = row32 > (lane32 & 31)
        m_even = (lane16 & 32) == 0
        m_lo = lane16 < 64
        m_mid = (lane16 >= 32) & (lane16 < 96)
        sub8 = lax.broadcasted_iota(jnp.int32, (8, 128), 0)

        def sel(mask, a, b):
            if a is None and b is None:
                return None
            z = jnp.zeros((16, 128), u32)
            return jnp.where(mask, z if a is None else a, z if b is None else b)

        def tmin_of(b):
            return max(0, 8 - 4 * (qb + b)) if isinstance(qb, int) else 0

        def qk(b, g, js):
            tmin = tmin_of(b)
            u = (lane16 + (128 - (80 * g) % 128)) & 127
            hm = [(u >= 20 * hh) & (u < 20 * hh + 20) for hh in range(4)]
            res = []
            for j in js:
                q32 = qext[g, _ds((lb + b) * 64 + 16 * j, 16, 16), :]
                w = jnp.concatenate([jnp.where(hm[(p - j) % 4], q32, u32(0)) for p in range(4)], axis=0)
                i0 = max(0, tmin - j)
                nblk = 9 - i0
                kj = kext[g, _ds((qb + b) * 64 - 128 + 16 * (j + i0), 16 * nblk, 16), :]
                s = lax.dot_general(_b16(kj), _b16(w), NT, preferred_element_type=f32)
                last = s[32 * (nblk - 1):32 * nblk]
                if i0 == 0:
                    sf = jnp.where(tri, s[0:32], last)
                    mid0 = 1
                else:
                    sf = jnp.where(tri, NEGBIG, last)
                    mid0 = 0
                m = jnp.max(sf, axis=0, keepdims=True)
                sm = None
                if nblk - 1 > mid0:
                    sm = s[32 * mid0:32 * (nblk - 1)]
                    m = jnp.maximum(m, jnp.max(sm, axis=0, keepdims=True))
                res.append((sf, sm, m, i0))
            return res

        def pv(b, g, res):
            tmin = tmin_of(b)
            A = [[None] * 9 for _ in range(4)]

            def make(j, ii, dep):
                sf, sm, m, i0 = res[j]
                if ii < i0 or ii > 8 or A[j][ii] is not None:
                    return
                if dep is not None:
                    m8 = pltpu.bitcast(jnp.broadcast_to(m, (8, 128)), u32) | dep
                    m8 = pltpu.bitcast(m8, f32)
                    m = jnp.concatenate([m8, m8, m8, m8], axis=0)
                if ii == 8 or ii == 0:
                    pf = jnp.exp2(sf - m)
                    if i0 == 0:
                        A[j][0] = _pack32(jnp.where(tri, pf, 0.0))
                        A[j][8] = _pack32(jnp.where(tri, 0.0, pf))
                    else:
                        A[j][8] = _pack32(pf)
                else:
                    ib = max(i0, 1)
                    A[j][ii] = _pack32(jnp.exp2(sm[32 * (ii - ib):32 * (ii - ib) + 32] - m))

            B = [[], [], [], []]
            for t in range(tmin, 12):
                dep = None
                if chain and len(B[3]) >= chain:
                    dep = B[3][-chain][8:16] >> 31
                for j in range(4):
                    if t - j >= 0:
                        make(j, t - j, dep)
                a = [A[j][t - j] if 0 <= t - j <= 8 else None for j in range(4)]
                d0 = sel(m_even, a[0], a[1]); d1 = sel(m_even, a[1], a[0])
                d2 = sel(m_even, a[2], a[3]); d3 = sel(m_even, a[3], a[2])
                B[0].append(sel(m_lo, d0, d2)); B[2].append(sel(m_lo, d2, d0))
                B[1].append(sel(m_mid, d1, d3)); B[3].append(sel(m_mid, d3, d1))
            kb0 = tmin // 4
            vbase = qb + b - 2
            sub8w = lax.broadcasted_iota(jnp.int32, (8, 128 * (3 - kb0)), 0)
            outs = []
            for hh in range(4):
                pT = _b16(jnp.concatenate(B[hh], axis=0))
                r0 = 40 * g + 8 * hh
                va = jnp.concatenate([vt[vbase + ii, r0:r0 + 8, :] for ii in range(kb0, 3)], axis=1)
                vb = jnp.concatenate([vt[vbase + ii, r0 + 8:r0 + 16, :] for ii in range(kb0, 3)], axis=1)
                if hh < 2:
                    vb = jnp.where(sub8w >= 4, u32(ONE2), vb)
                else:
                    va = jnp.where(sub8w < 4, u32(ONE2), va)
                vw = _b16(jnp.concatenate([va, vb], axis=0))
                o = jnp.dot(vw, pT, preferred_element_type=f32)
                if hh < 2:
                    den = o[24:32]; val = o[0:24]
                else:
                    den = o[0:8]; val = o[8:32]
                inv = 1.0 / den
                val = val * jnp.concatenate([inv, inv, inv], axis=0)
                if hh:
                    val = pltpu.roll(val, 128 - 32 * hh, 1)
                outs.append(val)
            v2 = jnp.where(sub8 < 4, outs[0][16:24], outs[1][0:8])
            v7 = jnp.where(sub8 < 4, outs[2][16:24], outs[3][0:8])
            return jnp.concatenate([outs[0][0:16], v2, outs[1][8:24], outs[2][0:16], v7, outs[3][8:24]], axis=0)

        items = [(b, g) for b in range(nqb) for g in range(NG)]
        og = {}
        prev = None
        for n, it in enumerate(items):
            rs = []
            for ch in patterns[n % len(patterns)]:
                if ch == 'F':
                    run_fill(pieces, 1, keep + 2)
                elif ch == 'P':
                    if prev is not None:
                        og[prev[0]] = pv(prev[0][0], prev[0][1], prev[1])
                elif ch == 'a':
                    rs += qk(it[0], it[1], (0, 1))
                elif ch == 'b':
                    rs += qk(it[0], it[1], (2, 3))
                else:
                    rs += qk(it[0], it[1], (int(ch),))
            prev = (it, rs)
        run_fill(pieces, len(pieces), keep + 1)
        og[prev[0]] = pv(prev[0][0], prev[0][1], prev[1])
        run_fill(pieces, len(pieces), keep)
        return jnp.concatenate([jnp.concatenate([og[(b, g)] for g in range(NG)], axis=0) for b in range(nqb)], axis=1)

    def wo_pieces(qb, lb, nqb, ot):
        st = {'h': []}

        def part(n):
            if 'o' not in st:
                st['o'] = ot.T.astype(bf16)
            st['h'].append(x_v[_ds(qb * QB, nqb * QB, QB), 128 * n:128 * n + 128].astype(f32)
                           + jnp.dot(st['o'], wo_v[:, 128 * n:128 * n + 128], preferred_element_type=f32))

        def get_hn():
            if 'hn' not in st:
                st['hn'] = _u32(_ln(jnp.concatenate(st['h'], axis=1)).astype(bf16))
            return st['hn']

        def store():
            h_scr[_ds(lb * QB, nqb * QB, QB), :] = jnp.concatenate(st['h'], axis=1)
            hn_scr[_ds(lb * 64, nqb * 64, 64), :] = get_hn()

        return [P(part, n) for n in range(5)], get_hn, store

    def attn_block(qb, lb, nqb, pieces, patterns, mid=None):
        pieces = list(pieces)
        ot = attention(qb, lb, nqb, pieces, patterns, 2, CHAIN)
        wo, get_hn, store = wo_pieces(qb, lb, nqb, ot)
        for p in wo:
            p()
        run_fill(pieces, len(pieces), 0)
        store()
        if mid is not None:
            mid()
        for p in ffn_first(get_hn, lb, nqb):
            p()

    def mix(gu, qkv, w2):
        out = list(gu[0:2]); rest = list(gu[2:]); qkv = list(qkv)
        while rest or qkv:
            out += qkv[0:2]; qkv = qkv[2:]
            out += rest[0:2]; rest = rest[2:]
        return out + list(w2)

    def steady(i, carry):
        with scope("steady"):
            if ONLY != 's':
                xcopy(i + 1).wait()
            gu, w2, _ = ffn_rest((i - 1) * NB, 0, NB, False)
            kp, qp, vp, store, _ = qkv_pieces(i + 1)
            attn_block(i * NB, 0, NB, mix(gu, kp + qp + vp, w2), VAR, store)
        return carry

    if ONLY == 's':
        lax.fori_loop(1, NSTEP - 1, steady, 0)
        return

    for c in (xcopy(0), xcopy(1), cp_ka, cp_kb, cp_q, cp_v, cp_o, cp_1a, cp_3a, cp_1b, cp_3b, cp_2, xcopy(2)):
        c.start()

    k0, q0, v0, store0, ln0 = qkv_pieces(0)
    k1, q1, v1, store1, ln1 = qkv_pieces(1)
    with scope("pro_a"):
        xcopy(0).wait()
        ln0()
        xcopy(1).wait()
        ln1()
        cp_ka.wait()
        for n in range(KA):
            k0[n]()
            k1[n]()
    with scope("pro_b"):
        cp_kb.wait()
        for n in range(KA, 5):
            k0[n]()
            k1[n]()
    with scope("pro_c"):
        cp_q.wait()
        for p in q0:
            p()
    with scope("pro_d"):
        cp_v.wait()
        q1[0]()
        q1[1]()
        wv = wqkv_v[:, 2 * D:3 * D].astype(f32)
        wvt_v[...] = _u32(wv.T.astype(bf16))
        for p in v0:
            p()
        store0()
        fill = q1[2:] + v1
        ot0 = attention(0, 0, 1, fill, VAR0, 0, CHAIN0)
    with scope("pro_e"):
        cp_o.wait()
        cp_1a.wait()
        cp_3a.wait()
        wo0, get_hn0, st0 = wo_pieces(0, 0, 1, ot0)
        fill = wo0 + ffn_first(get_hn0, 0, 1)
        ot1 = attention(1, 1, 1, fill, VAR1, KEEP1, CHAIN0)
        st0()
        wo1, get_hn1, st1 = wo_pieces(1, 1, 1, ot1)
        for p in wo1:
            p()
        run_fill(fill, len(fill), 0)
        st1()
        store1()
        for p in ffn_first(get_hn1, 1, 1):
            p()
    with scope("wwait"):
        cp_1b.wait()
        cp_3b.wait()
        cp_2.wait()
    for i in range(3, NSTEP):
        xcopy(i).start()
    if ONLY == 'p':
        for i in range(2, NSTEP):
            xcopy(i).wait()
        return

    lax.fori_loop(1, NSTEP - 1, steady, 0)

    def epi1(b, carry):
        with scope("epi1"):
            gu, w2, _ = ffn_rest((NSTEP - 2) * NB + b, b, 1, False)
            attn_block((NSTEP - 1) * NB + b, b, 1, gu + w2, VAR7)
        return carry

    lax.fori_loop(0, NB, epi1, 0)

    with scope("epi2"):
        gu, w2, _ = ffn_rest((NSTEP - 1) * NB, 0, NB, True)
        for p in gu + w2:
            p()
    with scope("owait"):
        for i in range(NSTEP - 2):
            ocopy(i * NB, NB).wait()
        for b in range(NB):
            ocopy((NSTEP - 2) * NB + b, 1).wait()
        for n in range(5):
            ocopy_col((NSTEP - 1) * NB, NB, n).wait()


@jax.jit
def pallas_sequential_preLN__sliding_block__glu_gated_swiglu__prompt_kernel(A_x, A_wqkv, A_wo, B_x, B_w1, B_w3, B_w2):
    any_spec = pl.BlockSpec(memory_space=pl.ANY)
    return pl.pallas_call(
        kernel,
        in_specs=[any_spec] * 6,
        out_specs=any_spec,
        out_shape=jax.ShapeDtypeStruct((1, S, D), bf16),
        scratch_shapes=[
            pltpu.VMEM((S, D), bf16), pltpu.VMEM((S, D), bf16),
            pltpu.VMEM((D, 3 * D), bf16), pltpu.VMEM((D, D), bf16), pltpu.VMEM((F, D), bf16),
            pltpu.VMEM((F, D), bf16), pltpu.VMEM((F, D), bf16), pltpu.VMEM((D // 2, D), u32),
            pltpu.VMEM((NG, S // 2, 128), u32), pltpu.VMEM((S // 128, D // 2, 128), u32),
            pltpu.VMEM((NG, T // 2, 128), u32),
            pltpu.VMEM((T, D), f32), pltpu.VMEM((T // 2, D), u32), pltpu.VMEM((T // 2, FA), u32),
            pltpu.SemaphoreType.DMA((NW + NSTEP,)),
            pltpu.SemaphoreType.DMA((S // QB + 5,)),
        ],
        compiler_params=pltpu.CompilerParams(vmem_limit_bytes=100 * 1024 * 1024),
    )(A_x, A_wqkv, A_wo, B_w1.T, B_w3.T, B_w2)
```

```python
import contextlib
import functools
import math
import jax
import jax.numpy as jnp
from jax import lax
import jax.experimental.pallas as pl
import jax.experimental.pallas.tpu as pltpu

VAR = '0F1P2F3,0F1FP2F3'
VAR0 = 'abFP'
VAR1 = 'abPF'
VAR7 = 'aFbFPF'
NFIRST = int('5')
CHAIN = int('3')
CHAIN0 = int('4')
KA = int('2')
KEEP1 = int('3')
MIX = 'ggqq'
LNC1 = ''
LNC2 = ''
W2S = int('7')
OPEN = int('0')
CHAIN7 = int('3')
KEEP = int('2')
KEEP7 = int('2')
RES = int('1')
POST1 = int('2')
POST = int('1')
POST7 = int('1')
OPEN7 = int('0')
OPEN8 = int('1')
PRIO = ''
QORD = 'kkkkkqqqqqvvvvv'
XNI = int('0')
EMERGE = int('1')
ONELOOP = int('1')
W2S7 = int('7')
W2S8 = int('7')
LNC27 = ''
LNC20 = ''
XNI0 = int('0')
TSP = int('1')
C1 = int('2')
C2 = int('4')
SCOPES = int('0')
ONLY = ''

S, D, H, DH, WIN, F = 2048, 640, 32, 20, 256, 1728
T = 256
QB = 128
NB = T // QB
NG = 8
NSTEP = S // T
EPS = 1e-5
QSCALE = (DH ** -0.5) * math.log2(math.e)
FMAIN = 1664
FA = 128 * NFIRST
ONE2 = 0x3F803F80
NEGBIG = -1e30
NT = (((1,), (1,)), ((), ()))
f32 = jnp.float32
bf16 = jnp.bfloat16
u32 = jnp.uint32
NW = 10


def scope(name):
    return jax.named_scope(name) if SCOPES else contextlib.nullcontext()


def _ln(x):
    m = jnp.mean(x, axis=-1, keepdims=True)
    xc = x - m
    v = jnp.mean(xc * xc, axis=-1, keepdims=True)
    return xc * lax.rsqrt(v + EPS)


def _ln_chain(x, spec):
    if not spec:
        return _ln(x)
    rows, dist = [int(v) for v in spec.split(':')]
    outs = []
    rs = []
    for c in range(x.shape[0] // rows):
        xc = x[c * rows:(c + 1) * rows]
        x0 = xc[:, 0:128]
        if c >= dist:
            dep = pltpu.bitcast(jnp.broadcast_to(rs[c - dist], (rows, 128)), u32) >> 31
            x0 = pltpu.bitcast(pltpu.bitcast(x0, u32) | dep, f32)
        s = x0
        for t in range(1, 5):
            s = s + xc[:, 128 * t:128 * t + 128]
        m = jnp.sum(s, axis=-1, keepdims=True) * (1.0 / D)
        xm = xc - m
        v = jnp.mean(xm * xm, axis=-1, keepdims=True)
        r = lax.rsqrt(v + EPS)
        rs.append(r)
        outs.append(xm * r)
    return jnp.concatenate(outs, axis=0)


def _u32(x):
    return pltpu.bitcast(x, u32)


def _b16(x):
    return pltpu.bitcast(x, bf16)


def _pack32(x):
    n = x.shape[0] // 32
    return jnp.concatenate(
        [pltpu.pack_elementwise([x[32 * i:32 * i + 16], x[32 * i + 16:32 * i + 32]], packed_dtype=bf16).astype(u32)
         for i in range(n)], axis=0)


def _group_tile(tiles, g, lane):
    lo = 80 * g
    ta = lo // 128
    off = lo % 128
    if off + 80 <= 128:
        return tiles[ta]
    return jnp.where(lane >= off, tiles[ta], tiles[ta + 1])


def _silu_mul(g, u):
    hg = 0.5 * g
    return (hg * (1.0 + jnp.tanh(hg))) * u


def _ds(start, n, align):
    if isinstance(start, int):
        return pl.ds(start, n)
    return pl.ds(pl.multiple_of(start, align), n)


def kernel(x_hbm, wqkv_hbm, wo_hbm, w1_hbm, w3_hbm, w2_hbm, o_hbm,
           x_v, o_v, wqkv_v, wo_v, w1_v, w3_v, w2_v, wvt_v, kext, vt, qext, h_scr, hn_scr, act_scr,
           wsem, osem):
    P = functools.partial

    def wcopy(src, dst, k):
        return pltpu.make_async_copy(src, dst, wsem.at[k])

    def qcols(a, b, k):
        return wcopy(wqkv_hbm.at[:, a:b], wqkv_v.at[:, a:b], k)

    cp_c1 = qcols(0, 128 * C1, 0)
    cp_c2 = qcols(128 * C1, 128 * (C1 + C2), 1)
    cp_c3 = [qcols(128 * (C1 + C2), 3 * D, 2)]
    cp_m = [wcopy(wo_hbm, wo_v, 3), wcopy(w1_hbm.at[0:FA, :], w1_v.at[0:FA, :], 3),
            wcopy(w3_hbm.at[0:FA, :], w3_v.at[0:FA, :], 3)]
    cp_r = [wcopy(w1_hbm.at[FA:F, :], w1_v.at[FA:F, :], 4), wcopy(w3_hbm.at[FA:F, :], w3_v.at[FA:F, :], 4),
            wcopy(w2_hbm, w2_v, 4)]

    def xcopy(i, n, k):
        r = pl.ds(i * T, n * T)
        return pltpu.make_async_copy(x_hbm.at[0, r, :], x_v.at[r, :], wsem.at[k])

    def ocopy(qb, nqb):
        r = _ds(qb * QB, nqb * QB, QB)
        return pltpu.make_async_copy(o_v.at[r, :], o_hbm.at[0, r, :], osem.at[0])

    def ocopy_col(qb, nqb, n):
        r = _ds(qb * QB, nqb * QB, QB)
        return pltpu.make_async_copy(o_v.at[r, 128 * n:128 * n + 128], o_hbm.at[0, r, 128 * n:128 * n + 128],
                                     osem.at[0])

    def ffn_first(get_hn, lb, nqb, tsp=1):
        st = {}

        def gpart(c):
            st['g'] = lax.dot_general(_b16(get_hn()), w1_v[128 * c:128 * c + 128, :], NT, preferred_element_type=f32)

        def upart(c, nsplit):
            rp = nqb * 64 // nsplit
            for s in range(nsplit):
                u = lax.dot_general(_b16(get_hn()[s * rp:(s + 1) * rp]), w3_v[128 * c:128 * c + 128, :], NT,
                                    preferred_element_type=f32)
                act_scr[_ds(lb * 64 + s * rp, rp, rp), 128 * c:128 * c + 128] = _u32(
                    _silu_mul(st['g'][2 * s * rp:2 * (s + 1) * rp], u).astype(bf16))

        ps = []
        for c in range(NFIRST):
            ps += [P(gpart, c), P(upart, c, tsp if c == NFIRST - 1 else 1)]
        return ps

    def ffn_rest(qb, lb, nqb, colcopy, nopen, w2s):
        acts = []
        st = {}
        pr = _ds(lb * 64, nqb * 64, 64)
        fr = _ds(lb * QB, nqb * QB, QB)
        orow = _ds(qb * QB, nqb * QB, QB)

        def gpart(c):
            st['g'] = lax.dot_general(_b16(hn_scr[pr, :]), w1_v[128 * c:128 * c + 128, :], NT,
                                      preferred_element_type=f32)

        def upart(c):
            u = lax.dot_general(_b16(hn_scr[pr, :]), w3_v[128 * c:128 * c + 128, :], NT, preferred_element_type=f32)
            acts.append(_silu_mul(st['g'], u).astype(bf16))

        def tail():
            w = jnp.concatenate([w1_v[FMAIN:F, :], w3_v[FMAIN:F, :]], axis=0)
            r = lax.dot_general(_b16(hn_scr[pr, :]), w, NT, preferred_element_type=f32)
            acts.append(_silu_mul(r, pltpu.roll(r, 64, 1))[:, 0:64].astype(bf16))

        def w2a(n, ks):
            a = jnp.concatenate([_b16(act_scr[pr, :])] + acts[0:ks - NFIRST], axis=1)
            st['o', n] = h_scr[fr, 128 * n:128 * n + 128] + jnp.dot(
                a, w2_v[0:128 * ks, 128 * n:128 * n + 128], preferred_element_type=f32)

        def w2b(n, ks):
            a = jnp.concatenate(acts[ks - NFIRST:], axis=1)
            r = st['o', n] + jnp.dot(a, w2_v[128 * ks:F, 128 * n:128 * n + 128], preferred_element_type=f32)
            o_v[orow, 128 * n:128 * n + 128] = r.astype(bf16)
            if colcopy:
                ocopy_col(qb, nqb, n).start()
            elif n == 4:
                ocopy(qb, nqb).start()

        gu = []
        for c in range(NFIRST, 13):
            gu += [P(gpart, c), P(upart, c)]
        gu.append(tail)
        w2 = []
        opening = []
        for n in range(5):
            if n < nopen:
                opening.append(P(w2a, n, NFIRST))
                w2.append(P(w2b, n, NFIRST))
            else:
                w2 += [P(w2a, n, w2s), P(w2b, n, w2s)]
        return gu, w2, opening

    def qkv_pieces(i, spec='', xni_mode=XNI0):
        st = {'k': [None] * 5, 'q': [None] * 5, 'v': []}

        def ln1():
            if 'xn' not in st:
                xnf = _ln_chain(x_v[_ds(i * T, T, T), :].astype(f32), spec)
                st['xn'] = xnf.astype(bf16)
                if xni_mode == 1:
                    st['xni'] = _b16(_pack32(st['xn'].astype(f32)))
                elif xni_mode == 2:
                    xu = _pack32(xnf)
                    st['xni'] = _b16(xu)
                    parts = []
                    for c in range(T // 32):
                        blk = xu[16 * c:16 * c + 16]
                        for ix in range(2):
                            parts.append(pltpu.unpack_elementwise(blk, index=ix, packed_dtype=bf16, unpacked_dtype=f32))
                    st['xn'] = jnp.concatenate(parts, axis=0).astype(bf16)
                else:
                    st['xni'] = _b16(_pack32(xnf))

        def kpart(n):
            ln1()
            k = jnp.dot(st['xn'], wqkv_v[:, D + 128 * n:D + 128 * n + 128], preferred_element_type=f32)
            st['k'][n] = _u32(k.astype(bf16))

        def qpart(n):
            ln1()
            q = jnp.dot(st['xn'], wqkv_v[:, 128 * n:128 * n + 128], preferred_element_type=f32)
            st['q'][n] = _u32((q * QSCALE).astype(bf16))

        def vpart(n):
            ln1()
            v = lax.dot_general(_b16(wvt_v[64 * n:64 * n + 64, :]), st['xni'], NT, preferred_element_type=f32)
            st['v'].append(_u32(v.astype(bf16)))

        def store():
            lane = lax.broadcasted_iota(jnp.int32, (T // 2, 128), 1)
            for g in range(NG):
                qext[g] = _group_tile(st['q'], g, lane)
                kext[g, _ds(i * (T // 2), T // 2, T // 2), :] = _group_tile(st['k'], g, lane)
            for n in range(5):
                for b in range(NB):
                    vt[i * NB + b, 64 * n:64 * n + 64, :] = st['v'][n][:, b * 128:(b + 1) * 128]

        return ([P(kpart, n) for n in range(5)], [P(qpart, n) for n in range(5)], [P(vpart, n) for n in range(5)],
                store, ln1)

    def run_fill(pieces, n, keep):
        for _ in range(n):
            if len(pieces) > keep:
                pieces.pop(0)()

    def attention(qb, lb, nqb, pieces, patterns, keep, chain, post=1):
        patterns = patterns.split(',')
        lane16 = lax.broadcasted_iota(jnp.int32, (16, 128), 1)
        lane32 = lax.broadcasted_iota(jnp.int32, (32, 128), 1)
        row32 = lax.broadcasted_iota(jnp.int32, (32, 128), 0)
        tri = row32 > (lane32 & 31)
        m_even = (lane16 & 32) == 0
        m_lo = lane16 < 64
        m_mid = (lane16 >= 32) & (lane16 < 96)
        sub8 = lax.broadcasted_iota(jnp.int32, (8, 128), 0)

        def sel(mask, a, b):
            if a is None and b is None:
                return None
            z = jnp.zeros((16, 128), u32)
            return jnp.where(mask, z if a is None else a, z if b is None else b)

        def tmin_of(b):
            return max(0, 8 - 4 * (qb + b)) if isinstance(qb, int) else 0

        def qk(b, g, js):
            tmin = tmin_of(b)
            u = (lane16 + (128 - (80 * g) % 128)) & 127
            hm = [(u >= 20 * hh) & (u < 20 * hh + 20) for hh in range(4)]
            res = []
            for j in js:
                q32 = qext[g, _ds((lb + b) * 64 + 16 * j, 16, 16), :]
                w = jnp.concatenate([jnp.where(hm[(p - j) % 4], q32, u32(0)) for p in range(4)], axis=0)
                i0 = max(0, tmin - j)
                nblk = 9 - i0
                kj = kext[g, _ds((qb + b) * 64 - 128 + 16 * (j + i0), 16 * nblk, 16), :]
                s = lax.dot_general(_b16(kj), _b16(w), NT, preferred_element_type=f32)
                last = s[32 * (nblk - 1):32 * nblk]
                if i0 == 0:
                    sf = jnp.where(tri, s[0:32], last)
                    mid0 = 1
                else:
                    sf = jnp.where(tri, NEGBIG, last)
                    mid0 = 0
                m = jnp.max(sf, axis=0, keepdims=True)
                sm = None
                if nblk - 1 > mid0:
                    sm = s[32 * mid0:32 * (nblk - 1)]
                    m = jnp.maximum(m, jnp.max(sm, axis=0, keepdims=True))
                res.append((sf, sm, m, i0))
            return res

        def pv(b, g, res):
            tmin = tmin_of(b)
            A = [[None] * 9 for _ in range(4)]

            def make(j, ii, dep):
                sf, sm, m, i0 = res[j]
                if ii < i0 or ii > 8 or A[j][ii] is not None:
                    return
                if dep is not None:
                    m8 = pltpu.bitcast(jnp.broadcast_to(m, (8, 128)), u32) | dep
                    m8 = pltpu.bitcast(m8, f32)
                    m = jnp.concatenate([m8, m8, m8, m8], axis=0)
                if ii == 8 or ii == 0:
                    pf = jnp.exp2(sf - m)
                    if i0 == 0:
                        A[j][0] = _pack32(jnp.where(tri, pf, 0.0))
                        A[j][8] = _pack32(jnp.where(tri, 0.0, pf))
                    else:
                        A[j][8] = _pack32(pf)
                else:
                    ib = max(i0, 1)
                    A[j][ii] = _pack32(jnp.exp2(sm[32 * (ii - ib):32 * (ii - ib) + 32] - m))

            B = [[], [], [], []]
            for t in range(tmin, 12):
                dep = None
                if chain and len(B[3]) >= chain:
                    dep = B[3][-chain][8:16] >> 31
                for j in range(4):
                    if t - j >= 0:
                        make(j, t - j, dep)
                a = [A[j][t - j] if 0 <= t - j <= 8 else None for j in range(4)]
                d0 = sel(m_even, a[0], a[1]); d1 = sel(m_even, a[1], a[0])
                d2 = sel(m_even, a[2], a[3]); d3 = sel(m_even, a[3], a[2])
                B[0].append(sel(m_lo, d0, d2)); B[2].append(sel(m_lo, d2, d0))
                B[1].append(sel(m_mid, d1, d3)); B[3].append(sel(m_mid, d3, d1))
            kb0 = tmin // 4
            vbase = qb + b - 2
            sub8w = lax.broadcasted_iota(jnp.int32, (8, 128 * (3 - kb0)), 0)
            outs = []
            for hh in range(4):
                pT = _b16(jnp.concatenate(B[hh], axis=0))
                r0 = 40 * g + 8 * hh
                va = jnp.concatenate([vt[vbase + ii, r0:r0 + 8, :] for ii in range(kb0, 3)], axis=1)
                vb = jnp.concatenate([vt[vbase + ii, r0 + 8:r0 + 16, :] for ii in range(kb0, 3)], axis=1)
                if hh < 2:
                    vb = jnp.where(sub8w >= 4, u32(ONE2), vb)
                else:
                    va = jnp.where(sub8w < 4, u32(ONE2), va)
                vw = _b16(jnp.concatenate([va, vb], axis=0))
                o = jnp.dot(vw, pT, preferred_element_type=f32)
                if hh < 2:
                    den = o[24:32]; val = o[0:24]
                else:
                    den = o[0:8]; val = o[8:32]
                inv = 1.0 / den
                val = val * jnp.concatenate([inv, inv, inv], axis=0)
                if hh:
                    val = pltpu.roll(val, 128 - 32 * hh, 1)
                outs.append(val)
            v2 = jnp.where(sub8 < 4, outs[0][16:24], outs[1][0:8])
            v7 = jnp.where(sub8 < 4, outs[2][16:24], outs[3][0:8])
            return jnp.concatenate([outs[0][0:16], v2, outs[1][8:24], outs[2][0:16], v7, outs[3][8:24]], axis=0)

        items = [(b, g) for b in range(nqb) for g in range(NG)]
        og = {}
        prev = None
        for n, it in enumerate(items):
            rs = []
            for ch in patterns[n % len(patterns)]:
                if ch == 'F':
                    run_fill(pieces, 1, keep + post + 1)
                elif ch == 'P':
                    if prev is not None:
                        og[prev[0]] = pv(prev[0][0], prev[0][1], prev[1])
                elif ch == 'a':
                    rs += qk(it[0], it[1], (0, 1))
                elif ch == 'b':
                    rs += qk(it[0], it[1], (2, 3))
                else:
                    rs += qk(it[0], it[1], (int(ch),))
            prev = (it, rs)
        run_fill(pieces, len(pieces), keep + post)
        og[prev[0]] = pv(prev[0][0], prev[0][1], prev[1])
        run_fill(pieces, len(pieces), keep)
        return jnp.concatenate([jnp.concatenate([og[(b, g)] for g in range(NG)], axis=0) for b in range(nqb)], axis=1)

    def wo_pieces(qb, lb, nqb, ot, lnc):
        st = {'h': []}

        def part(n):
            if 'o' not in st:
                st['o'] = ot.T.astype(bf16)
            st['h'].append(x_v[_ds(qb * QB, nqb * QB, QB), 128 * n:128 * n + 128].astype(f32)
                           + jnp.dot(st['o'], wo_v[:, 128 * n:128 * n + 128], preferred_element_type=f32))

        def get_hn():
            if 'hn' not in st:
                st['hn'] = _u32(_ln_chain(jnp.concatenate(st['h'], axis=1), lnc).astype(bf16))
            return st['hn']

        def store():
            h_scr[_ds(lb * QB, nqb * QB, QB), :] = jnp.concatenate(st['h'], axis=1)
            hn_scr[_ds(lb * 64, nqb * 64, 64), :] = get_hn()

        return [P(part, n) for n in range(5)], get_hn, store

    def attn_block(qb, lb, nqb, pieces, patterns, keep, chain, post, lnc, mid=None):
        pieces = list(pieces)
        ot = attention(qb, lb, nqb, pieces, patterns, keep, chain, post)
        wo, get_hn, store = wo_pieces(qb, lb, nqb, ot, lnc)
        for p in wo:
            p()
        run_fill(pieces, len(pieces), 0)
        store()
        if mid is not None:
            mid()
        for p in ffn_first(get_hn, lb, nqb, TSP if nqb == NB else 1):
            p()

    def mix(gu, qkv, w2):
        gu = list(gu); qkv = list(qkv)
        head, _, cyc = MIX.partition(':')
        if not cyc:
            head, cyc = '', head
        out = []
        n = 0
        seq = head
        while gu or qkv:
            ch = head[n] if n < len(head) else cyc[(n - len(head)) % len(cyc)]
            n += 1
            src_list = gu if ch == 'g' else qkv
            if src_list:
                out.append(src_list.pop(0))
        return out + list(w2)

    def steady(i, carry):
        with scope("steady"):
            if ONLY != 's':
                @pl.when(i == 2)
                def _():
                    xcopy(3, NSTEP - 3, 0).wait()
            gu, w2, opening = ffn_rest((i - 1) * NB, 0, NB, False, OPEN, W2S)
            kp, qp, vp, store, _ = qkv_pieces(i + 1, LNC1, XNI)
            for p in opening:
                p()
            dd = {'k': list(kp), 'q': list(qp), 'v': list(vp)}
            attn_block(i * NB, 0, NB, mix(gu, [dd[c].pop(0) for c in QORD], w2), VAR, KEEP, CHAIN, POST, LNC2, store)
        return carry

    def epi1(b, carry):
        with scope("epi1"):
            gu, w2, opening = ffn_rest((NSTEP - 2) * NB + b, b, 1, False, OPEN7, W2S7)
            for p in opening:
                p()
            attn_block((NSTEP - 1) * NB + b, b, 1, gu + w2, VAR7, KEEP7, CHAIN7, POST7, LNC27)
            if EMERGE:
                gu, w2, opening = ffn_rest((NSTEP - 1) * NB + b, b, 1, True, 0, W2S8)
                for p in gu + w2:
                    p()
        return carry

    if ONLY == 'e':
        lax.fori_loop(0, NB, epi1, 0)
        return

    if ONLY == 's':
        lax.fori_loop(1, NSTEP - 1, steady, 0)
        return

    def prologue():
        for n, c in enumerate([xcopy(0, 1, 5), xcopy(1, 1, 6), cp_c1, cp_c2] + cp_c3 + cp_m + cp_r + [xcopy(2, 1, 4)]):
            c.start(priority=int(PRIO[n]) if PRIO else 0)

        k0, q0, v0, store0, ln0 = qkv_pieces(0)
        k1, q1, v1, store1, ln1 = qkv_pieces(1)
        with scope("pro_a"):
            with scope("w_x0"):
                xcopy(0, 1, 5).wait()
            ln0()
            with scope("w_x1"):
                xcopy(1, 1, 6).wait()
            ln1()
            with scope("w_c1"):
                cp_c1.wait()
            qk0 = q0 + k0
            qk1 = q1 + k1
            for n in range(C1):
                qk0[n]()
                qk1[n]()
        with scope("pro_b"):
            with scope('w_c2'):
                cp_c2.wait()
            for n in range(C1, C1 + C2):
                qk0[n]()
                qk1[n]()
        with scope("pro_d"):
            with scope('w_c3'):
                for c in cp_c3:
                    c.wait()
            for p in qk0[C1 + C2:]:
                p()
            wv = wqkv_v[:, 2 * D:3 * D].astype(f32)
            wvt_v[...] = _u32(wv.T.astype(bf16))
            for p in v0:
                p()
            store0()
            fill = qk1[C1 + C2:] + v1
            ot0 = attention(0, 0, 1, fill, VAR0, RES, CHAIN0)
        with scope("pro_e"):
            with scope('w_m'):
                for c in cp_m:
                    c.wait()
            wo0, get_hn0, st0 = wo_pieces(0, 0, 1, ot0, LNC20)
            fill = wo0 + fill + ffn_first(get_hn0, 0, 1)
            ot1 = attention(1, 1, 1, fill, VAR1, KEEP1, CHAIN0, POST1)
            st0()
            wo1, get_hn1, st1 = wo_pieces(1, 1, 1, ot1, LNC20)
            for p in wo1:
                p()
            run_fill(fill, len(fill), 0)
            st1()
            store1()
            for p in ffn_first(get_hn1, 1, 1):
                p()
        with scope("wwait"):
            for c in cp_r:
                c.wait()
            xcopy(2, 1, 4).wait()
        xcopy(3, NSTEP - 3, 0).start()
    if ONLY == 'p':
        prologue()
        xcopy(3, NSTEP - 3, 0).wait()

        def sink(i, c):
            r = pl.ds(pl.multiple_of(i * 8, 8), 8)
            a = (kext[i, r, :] + vt[i, r, :] + qext[i, r, :] + hn_scr[r, 0:128] + act_scr[r, 0:128] + wvt_v[r, 0:128]
                 + pltpu.bitcast(h_scr[r, 0:128], u32))
            o_v[0:16, 0:128] = _b16(a)
            return c
        lax.fori_loop(0, 2, sink, 0)
        ocopy(0, 1).start()
        ocopy(0, 1).wait()
        return


    if ONELOOP:
        def step(i, carry):
            @pl.when(i == 0)
            def _():
                prologue()

            @pl.when((i > 0) & (i < NSTEP - 1))
            def _():
                steady(i, 0)

            @pl.when(i >= NSTEP - 1)
            def _():
                epi1(i - (NSTEP - 1), 0)
            return carry
        lax.fori_loop(0, NSTEP + 1, step, 0)
    else:
        prologue()
        lax.fori_loop(1, NSTEP - 1, steady, 0)
        lax.fori_loop(0, NB, epi1, 0)

    with scope("owait"):
        for i in range(NSTEP - 2):
            ocopy(i * NB, NB).wait()
        for b in range(NB):
            ocopy((NSTEP - 2) * NB + b, 1).wait()
        for n in range(5):
            if EMERGE:
                for b in range(NB):
                    ocopy_col((NSTEP - 1) * NB + b, 1, n).wait()
            else:
                ocopy_col((NSTEP - 1) * NB, NB, n).wait()


@jax.jit
def pallas_sequential_preLN__sliding_block__glu_gated_swiglu__prompt_kernel(A_x, A_wqkv, A_wo, B_x, B_w1, B_w3, B_w2):
    any_spec = pl.BlockSpec(memory_space=pl.ANY)
    return pl.pallas_call(
        kernel,
        in_specs=[any_spec] * 6,
        out_specs=any_spec,
        out_shape=jax.ShapeDtypeStruct((1, S, D), bf16),
        scratch_shapes=[
            pltpu.VMEM((S, D), bf16), pltpu.VMEM((S, D), bf16),
            pltpu.VMEM((D, 3 * D), bf16), pltpu.VMEM((D, D), bf16), pltpu.VMEM((F, D), bf16),
            pltpu.VMEM((F, D), bf16), pltpu.VMEM((F, D), bf16), pltpu.VMEM((D // 2, D), u32),
            pltpu.VMEM((NG, S // 2, 128), u32), pltpu.VMEM((S // 128, D // 2, 128), u32),
            pltpu.VMEM((NG, T // 2, 128), u32),
            pltpu.VMEM((T, D), f32), pltpu.VMEM((T // 2, D), u32), pltpu.VMEM((T // 2, FA), u32),
            pltpu.SemaphoreType.DMA((7,)),
            pltpu.SemaphoreType.DMA((1,)),
        ],
        compiler_params=pltpu.CompilerParams(vmem_limit_bytes=100 * 1024 * 1024),
    )(A_x, A_wqkv, A_wo, B_w1.T, B_w3.T, B_w2)
```

```python
import functools
import math

import jax
import jax.numpy as jnp
from jax import lax
import jax.experimental.pallas as pl
import jax.experimental.pallas.tpu as pltpu

S, D, H, DH, WIN, F = 2048, 640, 32, 20, 256, 1728
T = 256
QB = 128
NB = T // QB
NG = H // 4
NSTEP = S // T
EPS = 1e-5
QSCALE = (DH ** -0.5) * math.log2(math.e)
FMAIN = 1664
NFIRST = 7
FA = 128 * NFIRST
C1, C2 = 2, 4
ONE2 = 0x3F803F80
NEGBIG = -1e30
NT = (((1,), (1,)), ((), ()))
f32 = jnp.float32
bf16 = jnp.bfloat16
u32 = jnp.uint32

PAT_STEADY = ('aFbPF',)
PAT_LAST = ('aFbPF', 'aFbPF', 'aFbPF', 'abFFPF')
PAT_QB0 = ('abFP',)
PAT_QB1 = ('abPF', 'abFFP')


def _ln(x):
    m = jnp.mean(x, axis=-1, keepdims=True)
    xc = x - m
    v = jnp.mean(xc * xc, axis=-1, keepdims=True)
    return xc * lax.rsqrt(v + EPS)


def _ln_chained(x, rows, dist):
    outs = []
    rs = []
    for c in range(x.shape[0] // rows):
        xc = x[c * rows:(c + 1) * rows]
        x0 = xc[:, 0:128]
        if c >= dist:
            dep = pltpu.bitcast(jnp.broadcast_to(rs[c - dist], (rows, 128)), u32) >> 31
            x0 = pltpu.bitcast(pltpu.bitcast(x0, u32) | dep, f32)
        s = x0
        for t in range(1, 5):
            s = s + xc[:, 128 * t:128 * t + 128]
        m = jnp.sum(s, axis=-1, keepdims=True) * (1.0 / D)
        xm = xc - m
        v = jnp.mean(xm * xm, axis=-1, keepdims=True)
        r = lax.rsqrt(v + EPS)
        rs.append(r)
        outs.append(xm * r)
    return jnp.concatenate(outs, axis=0)


def _u32(x):
    return pltpu.bitcast(x, u32)


def _b16(x):
    return pltpu.bitcast(x, bf16)


def _pack32(x):
    n = x.shape[0] // 32
    xi = pltpu.bitcast(x, u32)
    return jnp.concatenate(
        [(xi[32 * i:32 * i + 16] >> 16) | (xi[32 * i + 16:32 * i + 32] & u32(0xFFFF0000)) for i in range(n)], axis=0)


def _group_tile(tiles, g, lane):
    lo = 80 * g
    ta = lo // 128
    off = lo % 128
    if off + 80 <= 128:
        return tiles[ta]
    return jnp.where(lane >= off, tiles[ta], tiles[ta + 1])


def _silu_mul(g, u):
    hg = 0.5 * g
    return (hg * (1.0 + jnp.tanh(hg))) * u


def _ds(start, n, align):
    if isinstance(start, int):
        return pl.ds(start, n)
    return pl.ds(pl.multiple_of(start, align), n)


def _kernel(x_hbm, wqkv_hbm, wo_hbm, w1_hbm, w3_hbm, w2_hbm, o_hbm,
            x_v, o_v, wqkv_v, wo_v, w1_v, w3_v, w2_v, wvt_v, kext, vt, qext, h_scr, hn_scr, act_scr,
            wsem, osem):
    P = functools.partial

    def wcopy(src, dst, k):
        return pltpu.make_async_copy(src, dst, wsem.at[k])

    def qcols(a, b, k):
        return wcopy(wqkv_hbm.at[:, a:b], wqkv_v.at[:, a:b], k)

    def xcopy(i, n, k):
        r = pl.ds(i * T, n * T)
        return pltpu.make_async_copy(x_hbm.at[0, r, :], x_v.at[r, :], wsem.at[k])

    def ocopy(qb, nqb):
        r = _ds(qb * QB, nqb * QB, QB)
        return pltpu.make_async_copy(o_v.at[r, :], o_hbm.at[0, r, :], osem.at[0])

    def ocopy_col(qb, nqb, n):
        r = _ds(qb * QB, nqb * QB, QB)
        return pltpu.make_async_copy(o_v.at[r, 128 * n:128 * n + 128], o_hbm.at[0, r, 128 * n:128 * n + 128],
                                     osem.at[0])

    def ffn_first(get_hn, lb, nqb):
        st = {}

        def gpart(c):
            st['g'] = lax.dot_general(_b16(get_hn()), w1_v[128 * c:128 * c + 128, :], NT, preferred_element_type=f32)

        def upart(c):
            u = lax.dot_general(_b16(get_hn()), w3_v[128 * c:128 * c + 128, :], NT, preferred_element_type=f32)
            act_scr[_ds(lb * 64, nqb * 64, 64), 128 * c:128 * c + 128] = _u32(_silu_mul(st['g'], u).astype(bf16))

        ps = []
        for c in range(NFIRST):
            ps += [P(gpart, c), P(upart, c)]
        return ps

    def ffn_rest(qb, lb, nqb, colcopy, nopen, w2s):
        acts = []
        st = {}
        pr = _ds(lb * 64, nqb * 64, 64)
        fr = _ds(lb * QB, nqb * QB, QB)
        orow = _ds(qb * QB, nqb * QB, QB)

        def gpart(c):
            st['g'] = lax.dot_general(_b16(hn_scr[pr, :]), w1_v[128 * c:128 * c + 128, :], NT,
                                      preferred_element_type=f32)

        def upart(c):
            u = lax.dot_general(_b16(hn_scr[pr, :]), w3_v[128 * c:128 * c + 128, :], NT, preferred_element_type=f32)
            acts.append(_silu_mul(st['g'], u).astype(bf16))

        def tail():
            w = jnp.concatenate([w1_v[FMAIN:F, :], w3_v[FMAIN:F, :]], axis=0)
            r = lax.dot_general(_b16(hn_scr[pr, :]), w, NT, preferred_element_type=f32)
            acts.append(_silu_mul(r, pltpu.roll(r, 64, 1))[:, 0:64].astype(bf16))

        def w2a(n, ks):
            a = jnp.concatenate([_b16(act_scr[pr, :])] + acts[0:ks - NFIRST], axis=1)
            st['o', n] = h_scr[fr, 128 * n:128 * n + 128] + jnp.dot(
                a, w2_v[0:128 * ks, 128 * n:128 * n + 128], preferred_element_type=f32)

        def w2b(n, ks):
            a = jnp.concatenate(acts[ks - NFIRST:], axis=1)
            r = st['o', n] + jnp.dot(a, w2_v[128 * ks:F, 128 * n:128 * n + 128], preferred_element_type=f32)
            o_v[orow, 128 * n:128 * n + 128] = r.astype(bf16)
            if colcopy:
                ocopy_col(qb, nqb, n).start()
            elif n == 4:
                ocopy(qb, nqb).start()

        gu = []
        for c in range(NFIRST, 13):
            gu += [P(gpart, c), P(upart, c)]
        gu.append(tail)
        w2 = []
        opening = []
        for n in range(5):
            if n < nopen:
                opening.append(P(w2a, n, NFIRST))
                w2.append(P(w2b, n, NFIRST))
            else:
                w2 += [P(w2a, n, w2s), P(w2b, n, w2s)]
        return gu, w2, opening

    def qkv_pieces(i, tall_v):
        st = {'k': [None] * 5, 'q': [None] * 5}

        def ln1():
            if 'xn' not in st:
                st['xn'] = _ln(x_v[_ds(i * T, T, T), :].astype(f32)).astype(bf16)
                st['xni'] = _b16(_pack32(st['xn'].astype(f32)))

        def kpart(n):
            ln1()
            k = jnp.dot(st['xn'], wqkv_v[:, D + 128 * n:D + 128 * n + 128], preferred_element_type=f32)
            st['k'][n] = _u32(k.astype(bf16))

        def qpart(n):
            ln1()
            q = jnp.dot(st['xn'], wqkv_v[:, 128 * n:128 * n + 128], preferred_element_type=f32)
            st['q'][n] = _u32((q * QSCALE).astype(bf16))

        def vpart(n):
            ln1()
            v = lax.dot_general(_b16(wvt_v[64 * n:64 * n + 64, :]), st['xni'], NT, preferred_element_type=f32)
            vu = _u32(v.astype(bf16))
            for b in range(NB):
                st['v', 64 * n, 64, b] = vu[:, b * 128:(b + 1) * 128]

        def vpart_tall(n):
            ln1()
            m, b = n // NB, n % NB
            v = lax.dot_general(_b16(wvt_v[160 * m:160 * m + 160, :]), st['xni'][b * QB:(b + 1) * QB], NT,
                                preferred_element_type=f32)
            st['v', 160 * m, 160, b] = _u32(v.astype(bf16))

        def store(what='qkv'):
            lane = lax.broadcasted_iota(jnp.int32, (T // 2, 128), 1)
            for g in range(NG):
                if 'q' in what:
                    qext[g] = _group_tile(st['q'], g, lane)
                if 'k' in what:
                    kext[g, _ds(i * (T // 2), T // 2, T // 2), :] = _group_tile(st['k'], g, lane)
            if 'v' in what:
                for key in [kk for kk in st if isinstance(kk, tuple)]:
                    _, r0, nr, b = key
                    vt[i * NB + b, r0:r0 + nr, :] = st.pop(key)

        vp = [P(vpart_tall, n) for n in range(4)] if tall_v else [P(vpart, n) for n in range(5)]
        return [P(kpart, n) for n in range(5)], [P(qpart, n) for n in range(5)], vp, store, ln1

    def run_fill(pieces, n, keep):
        for _ in range(n):
            if len(pieces) > keep:
                pieces.pop(0)()

    def attention(qb, lb, nqb, pieces, patterns, keep, chain, post):
        lane16 = lax.broadcasted_iota(jnp.int32, (16, 128), 1)
        lane32 = lax.broadcasted_iota(jnp.int32, (32, 128), 1)
        row32 = lax.broadcasted_iota(jnp.int32, (32, 128), 0)
        tri = row32 > (lane32 & 31)
        m_even = (lane16 & 32) == 0
        m_lo = lane16 < 64
        m_mid = (lane16 >= 32) & (lane16 < 96)
        sub8 = lax.broadcasted_iota(jnp.int32, (8, 128), 0)

        def sel(mask, a, b):
            if a is None and b is None:
                return None
            z = jnp.zeros((16, 128), u32)
            return jnp.where(mask, z if a is None else a, z if b is None else b)

        def tmin_of(b):
            return max(0, 8 - 4 * (qb + b)) if isinstance(qb, int) else 0

        def qk(b, g, js):
            tmin = tmin_of(b)
            u = (lane16 + (128 - (80 * g) % 128)) & 127
            hm = [(u >= 20 * hh) & (u < 20 * hh + 20) for hh in range(4)]
            res = []
            for j in js:
                q32 = qext[g, _ds((lb + b) * 64 + 16 * j, 16, 16), :]
                w = jnp.concatenate([jnp.where(hm[(p - j) % 4], q32, u32(0)) for p in range(4)], axis=0)
                i0 = max(0, tmin - j)
                nblk = 9 - i0
                kj = kext[g, _ds((qb + b) * 64 - 128 + 16 * (j + i0), 16 * nblk, 16), :]
                s = lax.dot_general(_b16(kj), _b16(w), NT, preferred_element_type=f32)
                last = s[32 * (nblk - 1):32 * nblk]
                if i0 == 0:
                    sf = jnp.where(tri, s[0:32], last)
                    mid0 = 1
                else:
                    sf = jnp.where(tri, NEGBIG, last)
                    mid0 = 0
                m = jnp.max(sf, axis=0, keepdims=True)
                sm = None
                if nblk - 1 > mid0:
                    sm = s[32 * mid0:32 * (nblk - 1)]
                    m = jnp.maximum(m, jnp.max(sm, axis=0, keepdims=True))
                res.append((sf, sm, m, i0))
            return res

        def pv(b, g, res):
            tmin = tmin_of(b)
            A = [[None] * 9 for _ in range(4)]

            def make(j, ii, dep):
                sf, sm, m, i0 = res[j]
                if ii < i0 or ii > 8 or A[j][ii] is not None:
                    return
                if dep is not None:
                    m8 = pltpu.bitcast(jnp.broadcast_to(m, (8, 128)), u32) | dep
                    m8 = pltpu.bitcast(m8, f32)
                    m = jnp.concatenate([m8, m8, m8, m8], axis=0)
                if ii == 8 or ii == 0:
                    pf = jnp.exp2(sf - m)
                    if i0 == 0:
                        A[j][0] = _pack32(jnp.where(tri, pf, 0.0))
                        A[j][8] = _pack32(jnp.where(tri, 0.0, pf))
                    else:
                        A[j][8] = _pack32(pf)
                else:
                    ib = max(i0, 1)
                    A[j][ii] = _pack32(jnp.exp2(sm[32 * (ii - ib):32 * (ii - ib) + 32] - m))

            B = [[], [], [], []]
            for t in range(tmin, 12):
                dep = None
                if len(B[3]) >= chain:
                    dep = B[3][-chain][8:16] >> 31
                for j in range(4):
                    if t - j >= 0:
                        make(j, t - j, dep)
                a = [A[j][t - j] if 0 <= t - j <= 8 else None for j in range(4)]
                d0 = sel(m_even, a[0], a[1])
                d1 = sel(m_even, a[1], a[0])
                d2 = sel(m_even, a[2], a[3])
                d3 = sel(m_even, a[3], a[2])
                B[0].append(sel(m_lo, d0, d2))
                B[2].append(sel(m_lo, d2, d0))
                B[1].append(sel(m_mid, d1, d3))
                B[3].append(sel(m_mid, d3, d1))
            kb0 = tmin // 4
            vbase = qb + b - 2
            sub8w = lax.broadcasted_iota(jnp.int32, (8, 128 * (3 - kb0)), 0)
            outs = []
            for hh in range(4):
                pT = _b16(jnp.concatenate(B[hh], axis=0))
                r0 = 40 * g + 8 * hh
                va = jnp.concatenate([vt[vbase + ii, r0:r0 + 8, :] for ii in range(kb0, 3)], axis=1)
                vb = jnp.concatenate([vt[vbase + ii, r0 + 8:r0 + 16, :] for ii in range(kb0, 3)], axis=1)
                if hh < 2:
                    vb = jnp.where(sub8w >= 4, u32(ONE2), vb)
                else:
                    va = jnp.where(sub8w < 4, u32(ONE2), va)
                vw = _b16(jnp.concatenate([va, vb], axis=0))
                o = jnp.dot(vw, pT, preferred_element_type=f32)
                if hh < 2:
                    den = o[24:32]
                    val = o[0:24]
                else:
                    den = o[0:8]
                    val = o[8:32]
                inv = 1.0 / den
                val = val * jnp.concatenate([inv, inv, inv], axis=0)
                if hh:
                    val = pltpu.roll(val, 128 - 32 * hh, 1)
                outs.append(val)
            v2 = jnp.where(sub8 < 4, outs[0][16:24], outs[1][0:8])
            v7 = jnp.where(sub8 < 4, outs[2][16:24], outs[3][0:8])
            return jnp.concatenate([outs[0][0:16], v2, outs[1][8:24], outs[2][0:16], v7, outs[3][8:24]], axis=0)

        items = [(b, g) for b in range(nqb) for g in range(NG)]
        og = {}
        prev = None
        for n, it in enumerate(items):
            rs = []
            for ch in patterns[n % len(patterns)]:
                if ch == 'F':
                    run_fill(pieces, 1, keep + post + 1)
                elif ch == 'P':
                    if prev is not None:
                        og[prev[0]] = pv(prev[0][0], prev[0][1], prev[1])
                elif ch == 'a':
                    rs += qk(it[0], it[1], (0, 1))
                elif ch == 'b':
                    rs += qk(it[0], it[1], (2, 3))
                else:
                    rs += qk(it[0], it[1], (int(ch),))
            prev = (it, rs)
        run_fill(pieces, len(pieces), keep + post)
        og[prev[0]] = pv(prev[0][0], prev[0][1], prev[1])
        run_fill(pieces, len(pieces), keep)
        return jnp.concatenate([jnp.concatenate([og[(b, g)] for g in range(NG)], axis=0) for b in range(nqb)], axis=1)

    def wo_pieces(qb, lb, nqb, ot, ln):
        st = {'h': []}

        def xpose():
            if 'o' not in st:
                st['o'] = ot.T.astype(bf16)

        def part(n):
            xpose()
            st['h'].append(x_v[_ds(qb * QB, nqb * QB, QB), 128 * n:128 * n + 128].astype(f32)
                           + jnp.dot(st['o'], wo_v[:, 128 * n:128 * n + 128], preferred_element_type=f32))

        def get_hn():
            if 'hn' not in st:
                st['hn'] = _u32(ln(jnp.concatenate(st['h'], axis=1)).astype(bf16))
            return st['hn']

        def store():
            h_scr[_ds(lb * QB, nqb * QB, QB), :] = jnp.concatenate(st['h'], axis=1)
            hn_scr[_ds(lb * 64, nqb * 64, 64), :] = get_hn()

        return [P(part, n) for n in range(5)], get_hn, store, xpose

    def attn_block(qb, lb, nqb, pieces, patterns, keep, chain, post, ln, mid=None):
        pieces = list(pieces)
        ot = attention(qb, lb, nqb, pieces, patterns, keep, chain, post)
        wo, get_hn, store, _ = wo_pieces(qb, lb, nqb, ot, ln)
        for p in wo:
            p()
        run_fill(pieces, len(pieces), 0)
        store()
        if mid is not None:
            mid()
        for p in ffn_first(get_hn, lb, nqb):
            p()

    def prologue():
        cp_c1 = qcols(0, 128 * C1, 0)
        cp_c2 = qcols(128 * C1, 128 * (C1 + C2), 1)
        cp_c3 = qcols(128 * (C1 + C2), 3 * D, 2)
        cp_m = [wcopy(wo_hbm, wo_v, 3), wcopy(w1_hbm.at[0:FA, :], w1_v.at[0:FA, :], 3),
                wcopy(w3_hbm.at[0:FA, :], w3_v.at[0:FA, :], 3)]
        cp_r = [wcopy(w1_hbm.at[FA:F, :], w1_v.at[FA:F, :], 4), wcopy(w3_hbm.at[FA:F, :], w3_v.at[FA:F, :], 4),
                wcopy(w2_hbm, w2_v, 4), xcopy(2, 1, 4)]
        cp_x0 = xcopy(0, 1, 5)
        cp_x1 = xcopy(1, 1, 6)
        for c in [cp_x0, cp_x1, cp_c1, cp_c2, cp_c3] + cp_m + cp_r:
            c.start()

        k0, q0, v0, store0, ln0 = qkv_pieces(0, False)
        k1, q1, v1, store1, ln1 = qkv_pieces(1, False)
        qk0 = q0 + k0
        qk1 = q1 + k1
        cp_x0.wait()
        ln0()
        cp_x1.wait()
        ln1()
        cp_c1.wait()
        for n in range(C1):
            qk0[n]()
            qk1[n]()
        cp_c2.wait()
        for n in range(C1, C1 + C2):
            qk0[n]()
            qk1[n]()
        cp_c3.wait()
        for p in qk0[C1 + C2:]:
            p()
        wvt_v[...] = _u32(wqkv_v[:, 2 * D:3 * D].astype(f32).T.astype(bf16))
        for p in v0:
            p()
        store0()
        fill = qk1[C1 + C2:] + v1
        ot0 = attention(0, 0, 1, fill, PAT_QB0, 1, 4, 1)
        wo0, get_hn0, st0, xp0 = wo_pieces(0, 0, 1, ot0, _ln)
        xp0()
        store1('kv')
        for c in cp_m:
            c.wait()
        fill = wo0 + fill + ffn_first(get_hn0, 0, 1)
        run_fill(fill, 2, 0)
        ot1 = attention(1, 1, 1, fill, PAT_QB1, 3, 6, 2)
        st0()
        wo1, get_hn1, st1, _ = wo_pieces(1, 1, 1, ot1, _ln)
        for p in wo1:
            p()
        run_fill(fill, len(fill), 0)
        st1()
        store1('qv')
        for p in ffn_first(get_hn1, 1, 1):
            p()
        for c in cp_r:
            c.wait()
        xcopy(3, NSTEP - 3, 0).start()

    def steady(i):
        @pl.when(i == 2)
        def _():
            xcopy(3, NSTEP - 3, 0).wait()

        gu, w2, opening = ffn_rest((i - 1) * NB, 0, NB, False, 1, 7)
        kp, qp, vp, store, _ = qkv_pieces(i + 1, True)
        for p in opening:
            p()
        qkv = kp + qp + vp
        fill = [gu.pop(0), qkv.pop(0)]
        n = 0
        while gu or qkv:
            src = gu if 'gqqg'[n % 4] == 'g' else qkv
            n += 1
            if src:
                fill.append(src.pop(0))
        attn_block(i * NB, 0, NB, fill + w2, PAT_STEADY, 2, 4, 1, _ln, store)

    def last(b):
        gu, w2, _ = ffn_rest((NSTEP - 2) * NB + b, b, 1, False, 0, 7)
        attn_block((NSTEP - 1) * NB + b, b, 1, gu + w2, PAT_LAST, 4, 5, 2, P(_ln_chained, rows=32, dist=2))
        gu, w2, _ = ffn_rest((NSTEP - 1) * NB + b, b, 1, True, 0, 8)
        for p in gu + w2:
            p()

    def step(i, carry):
        @pl.when(i == 0)
        def _():
            prologue()

        @pl.when((i > 0) & (i < NSTEP - 1))
        def _():
            steady(i)

        @pl.when(i >= NSTEP - 1)
        def _():
            last(i - (NSTEP - 1))
        return carry

    lax.fori_loop(0, NSTEP - 1 + NB, step, 0)

    for i in range(NSTEP - 2):
        ocopy(i * NB, NB).wait()
    for b in range(NB):
        ocopy((NSTEP - 2) * NB + b, 1).wait()
    for n in range(5):
        for b in range(NB):
            ocopy_col((NSTEP - 1) * NB + b, 1, n).wait()


@jax.jit
def pallas_sequential_preLN__sliding_block__glu_gated_swiglu__prompt_kernel(A_x, A_wqkv, A_wo, B_x, B_w1, B_w3, B_w2):
    del B_x
    any_spec = pl.BlockSpec(memory_space=pl.ANY)
    return pl.pallas_call(
        _kernel,
        in_specs=[any_spec] * 6,
        out_specs=any_spec,
        out_shape=jax.ShapeDtypeStruct((1, S, D), bf16),
        scratch_shapes=[
            pltpu.VMEM((S, D), bf16),
            pltpu.VMEM((S, D), bf16),
            pltpu.VMEM((D, 3 * D), bf16),
            pltpu.VMEM((D, D), bf16),
            pltpu.VMEM((F, D), bf16),
            pltpu.VMEM((F, D), bf16),
            pltpu.VMEM((F, D), bf16),
            pltpu.VMEM((D // 2, D), u32),
            pltpu.VMEM((NG, S // 2, 128), u32),
            pltpu.VMEM((S // 128, D // 2, 128), u32),
            pltpu.VMEM((NG, T // 2, 128), u32),
            pltpu.VMEM((T, D), f32),
            pltpu.VMEM((T // 2, D), u32),
            pltpu.VMEM((T // 2, FA), u32),
            pltpu.SemaphoreType.DMA((7,)),
            pltpu.SemaphoreType.DMA((1,)),
        ],
        compiler_params=pltpu.CompilerParams(vmem_limit_bytes=100 * 1024 * 1024),
    )(A_x, A_wqkv, A_wo, B_w1.T, B_w3.T, B_w2)
```

```python
import functools
import math

import jax
import jax.numpy as jnp
from jax import lax
import jax.experimental.pallas as pl
import jax.experimental.pallas.tpu as pltpu

S, D, H, DH, WIN, F = 2048, 640, 32, 20, 256, 1728
T = 256
QB = 128
NB = T // QB
NG = H // 4
NSTEP = S // T
EPS = 1e-5
QSCALE = (DH ** -0.5) * math.log2(math.e)
FMAIN = 1664
NFIRST = 7
FA = 128 * NFIRST
C1, C2 = 2, 4
ONE2 = 0x3F803F80
NEGBIG = -1e30
NT = (((1,), (1,)), ((), ()))
f32 = jnp.float32
bf16 = jnp.bfloat16
u32 = jnp.uint32

PAT_STEADY = ('aPFbF',) + ('aFbPF',) * 15
PAT_LAST = ('aFbFP', 'aFbPF', 'aFbPF', 'aFbPF', 'aFFPbF', 'aFbPF', '01F2P3F', 'abFPFF')
PAT_QB0 = ('aPbF', 'abP', 'abFP', 'abFP', 'aPb', 'abFP', 'abFFP', '0F12F3P')
PAT_QB1 = ('aPb', 'abFFP', 'abPF', '012F3P', 'FabP', '01F2F3P', '0F1F2F3P', 'abFFP')
FILL_STEADY = 'gkkkggkkgggqqgqqgggqvgggvvwvwwwwwwww'


def _ln(x):
    m = jnp.mean(x, axis=-1, keepdims=True)
    xc = x - m
    v = jnp.mean(xc * xc, axis=-1, keepdims=True)
    return xc * lax.rsqrt(v + EPS)


def _ln_chained(x, rows, dist):
    outs = []
    rs = []
    for c in range(x.shape[0] // rows):
        xc = x[c * rows:(c + 1) * rows]
        x0 = xc[:, 0:128]
        if c >= dist:
            dep = pltpu.bitcast(jnp.broadcast_to(rs[c - dist], (rows, 128)), u32) >> 31
            x0 = pltpu.bitcast(pltpu.bitcast(x0, u32) | dep, f32)
        s = x0
        for t in range(1, 5):
            s = s + xc[:, 128 * t:128 * t + 128]
        m = jnp.sum(s, axis=-1, keepdims=True) * (1.0 / D)
        xm = xc - m
        v = jnp.mean(xm * xm, axis=-1, keepdims=True)
        r = lax.rsqrt(v + EPS)
        rs.append(r)
        outs.append(xm * r)
    return jnp.concatenate(outs, axis=0)


def _u32(x):
    return pltpu.bitcast(x, u32)


def _b16(x):
    return pltpu.bitcast(x, bf16)


def _pack32(x):
    n = x.shape[0] // 32
    xi = pltpu.bitcast(x, u32)
    return jnp.concatenate(
        [(xi[32 * i:32 * i + 16] >> 16) | (xi[32 * i + 16:32 * i + 32] & u32(0xFFFF0000)) for i in range(n)], axis=0)


def _group_tile(tiles, g, lane):
    lo = 80 * g
    ta = lo // 128
    off = lo % 128
    if off + 80 <= 128:
        return tiles[ta]
    return jnp.where(lane >= off, tiles[ta], tiles[ta + 1])


def _silu_mul(g, u):
    hg = 0.5 * g
    return (hg * (1.0 + jnp.tanh(hg))) * u


def _ds(start, n, align):
    if isinstance(start, int):
        return pl.ds(start, n)
    return pl.ds(pl.multiple_of(start, align), n)


def _kernel(x_hbm, wqkv_hbm, wo_hbm, w1_hbm, w3_hbm, w2_hbm, o_hbm,
            x_v, o_v, wqkv_v, wo_v, w1_v, w3_v, w2_v, wvt_v, kext, vt, qext, h_scr, hn_scr, act_scr,
            wsem, osem):
    P = functools.partial

    def wcopy(src, dst, k):
        return pltpu.make_async_copy(src, dst, wsem.at[k])

    def qcols(a, b, k):
        return wcopy(wqkv_hbm.at[:, a:b], wqkv_v.at[:, a:b], k)

    def xcopy(i, n, k):
        r = pl.ds(i * T, n * T)
        return pltpu.make_async_copy(x_hbm.at[0, r, :], x_v.at[r, :], wsem.at[k])

    def ocopy(qb, nqb):
        r = _ds(qb * QB, nqb * QB, QB)
        return pltpu.make_async_copy(o_v.at[r, :], o_hbm.at[0, r, :], osem.at[0])

    def ocopy_col(qb, nqb, n):
        r = _ds(qb * QB, nqb * QB, QB)
        a, b = (0, 512) if n == 3 else (512, D)
        return pltpu.make_async_copy(o_v.at[r, a:b], o_hbm.at[0, r, a:b], osem.at[0])

    def ffn_first(get_hn, lb, nqb):
        st = {}

        def gpart(c):
            st['g'] = lax.dot_general(_b16(get_hn()), w1_v[128 * c:128 * c + 128, :], NT, preferred_element_type=f32)

        def upart(c):
            u = lax.dot_general(_b16(get_hn()), w3_v[128 * c:128 * c + 128, :], NT, preferred_element_type=f32)
            act_scr[_ds(lb * 64, nqb * 64, 64), 128 * c:128 * c + 128] = _u32(_silu_mul(st['g'], u).astype(bf16))

        ps = []
        for c in range(NFIRST):
            ps += [P(gpart, c), P(upart, c)]
        return ps

    def ffn_rest(qb, lb, nqb, colcopy, nopen, w2s):
        acts = []
        st = {}
        pr = _ds(lb * 64, nqb * 64, 64)
        fr = _ds(lb * QB, nqb * QB, QB)
        orow = _ds(qb * QB, nqb * QB, QB)

        def gpart(c):
            st['g'] = lax.dot_general(_b16(hn_scr[pr, :]), w1_v[128 * c:128 * c + 128, :], NT,
                                      preferred_element_type=f32)

        def upart(c):
            u = lax.dot_general(_b16(hn_scr[pr, :]), w3_v[128 * c:128 * c + 128, :], NT, preferred_element_type=f32)
            acts.append(_silu_mul(st['g'], u).astype(bf16))

        def tail():
            w = jnp.concatenate([w1_v[FMAIN:F, :], w3_v[FMAIN:F, :]], axis=0)
            r = lax.dot_general(_b16(hn_scr[pr, :]), w, NT, preferred_element_type=f32)
            acts.append(_silu_mul(r, pltpu.roll(r, 64, 1))[:, 0:64].astype(bf16))

        def w2a(n, ks):
            a = jnp.concatenate([_b16(act_scr[pr, :])] + acts[0:ks - NFIRST], axis=1)
            st['o', n] = h_scr[fr, 128 * n:128 * n + 128] + jnp.dot(
                a, w2_v[0:128 * ks, 128 * n:128 * n + 128], preferred_element_type=f32)

        def w2b(n, ks):
            a = jnp.concatenate(acts[ks - NFIRST:], axis=1)
            r = st['o', n] + jnp.dot(a, w2_v[128 * ks:F, 128 * n:128 * n + 128], preferred_element_type=f32)
            o_v[orow, 128 * n:128 * n + 128] = r.astype(bf16)
            if colcopy:
                if n >= 3:
                    ocopy_col(qb, nqb, n).start()
            elif n == 4:
                ocopy(qb, nqb).start()

        gu = []
        for c in range(NFIRST, 13):
            gu += [P(gpart, c), P(upart, c)]
        gu.append(tail)
        w2 = []
        opening = []
        for n in range(5):
            if n < nopen:
                opening.append(P(w2a, n, NFIRST))
                w2.append(P(w2b, n, NFIRST))
            else:
                w2 += [P(w2a, n, w2s), P(w2b, n, w2s)]
        return gu, w2, opening

    def qkv_pieces(i, tall_v):
        st = {'k': [None] * 5, 'q': [None] * 5}

        def ln1():
            if 'xn' not in st:
                st['xn'] = _ln(x_v[_ds(i * T, T, T), :].astype(f32)).astype(bf16)
                st['xni'] = _b16(_pack32(st['xn'].astype(f32)))

        def kpart(n):
            ln1()
            k = jnp.dot(st['xn'], wqkv_v[:, D + 128 * n:D + 128 * n + 128], preferred_element_type=f32)
            st['k'][n] = _u32(k.astype(bf16))

        def qpart(n):
            ln1()
            q = jnp.dot(st['xn'], wqkv_v[:, 128 * n:128 * n + 128], preferred_element_type=f32)
            st['q'][n] = _u32((q * QSCALE).astype(bf16))

        def vpart(n):
            ln1()
            v = lax.dot_general(_b16(wvt_v[64 * n:64 * n + 64, :]), st['xni'], NT, preferred_element_type=f32)
            vu = _u32(v.astype(bf16))
            for b in range(NB):
                st['v', 64 * n, 64, b] = vu[:, b * 128:(b + 1) * 128]

        def vpart_tall(n):
            ln1()
            m, b = n // NB, n % NB
            v = lax.dot_general(_b16(wvt_v[160 * m:160 * m + 160, :]), st['xni'][b * QB:(b + 1) * QB], NT,
                                preferred_element_type=f32)
            st['v', 160 * m, 160, b] = _u32(v.astype(bf16))

        def store(what='qkv'):
            lane = lax.broadcasted_iota(jnp.int32, (T // 2, 128), 1)
            for g in range(NG):
                if 'q' in what:
                    qext[g] = _group_tile(st['q'], g, lane)
                if 'k' in what:
                    kext[g, _ds(i * (T // 2), T // 2, T // 2), :] = _group_tile(st['k'], g, lane)
            if 'v' in what:
                for key in [kk for kk in st if isinstance(kk, tuple)]:
                    _, r0, nr, b = key
                    vt[i * NB + b, r0:r0 + nr, :] = st.pop(key)

        vp = [P(vpart_tall, n) for n in range(4)] if tall_v else [P(vpart, n) for n in range(5)]
        return [P(kpart, n) for n in range(5)], [P(qpart, n) for n in range(5)], vp, store, ln1

    def run_fill(pieces, n, keep):
        for _ in range(n):
            if len(pieces) > keep:
                pieces.pop(0)()

    def attention(qb, lb, nqb, pieces, patterns, keep, chain, post):
        lane16 = lax.broadcasted_iota(jnp.int32, (16, 128), 1)
        lane32 = lax.broadcasted_iota(jnp.int32, (32, 128), 1)
        row32 = lax.broadcasted_iota(jnp.int32, (32, 128), 0)
        tri = row32 > (lane32 & 31)
        m_even = (lane16 & 32) == 0
        m_lo = lane16 < 64
        m_mid = (lane16 >= 32) & (lane16 < 96)
        sub8 = lax.broadcasted_iota(jnp.int32, (8, 128), 0)

        def sel(mask, a, b):
            if a is None and b is None:
                return None
            z = jnp.zeros((16, 128), u32)
            return jnp.where(mask, z if a is None else a, z if b is None else b)

        def tmin_of(b):
            return max(0, 8 - 4 * (qb + b)) if isinstance(qb, int) else 0

        def qk(b, g, js):
            tmin = tmin_of(b)
            u = (lane16 + (128 - (80 * g) % 128)) & 127
            hm = [(u >= 20 * hh) & (u < 20 * hh + 20) for hh in range(4)]
            res = []
            for j in js:
                q32 = qext[g, _ds((lb + b) * 64 + 16 * j, 16, 16), :]
                w = jnp.concatenate([jnp.where(hm[(p - j) % 4], q32, u32(0)) for p in range(4)], axis=0)
                i0 = max(0, tmin - j)
                nblk = 9 - i0
                kj = kext[g, _ds((qb + b) * 64 - 128 + 16 * (j + i0), 16 * nblk, 16), :]
                s = lax.dot_general(_b16(kj), _b16(w), NT, preferred_element_type=f32)
                last = s[32 * (nblk - 1):32 * nblk]
                if i0 == 0:
                    sf = jnp.where(tri, s[0:32], last)
                    mid0 = 1
                else:
                    sf = jnp.where(tri, NEGBIG, last)
                    mid0 = 0
                m = jnp.max(sf, axis=0, keepdims=True)
                sm = None
                if nblk - 1 > mid0:
                    sm = s[32 * mid0:32 * (nblk - 1)]
                    m = jnp.maximum(m, jnp.max(sm, axis=0, keepdims=True))
                res.append((sf, sm, m, i0))
            return res

        def pv(b, g, res):
            tmin = tmin_of(b)
            A = [[None] * 9 for _ in range(4)]

            def make(j, ii, dep):
                sf, sm, m, i0 = res[j]
                if ii < i0 or ii > 8 or A[j][ii] is not None:
                    return
                if dep is not None:
                    m8 = pltpu.bitcast(jnp.broadcast_to(m, (8, 128)), u32) | dep
                    m8 = pltpu.bitcast(m8, f32)
                    m = jnp.concatenate([m8, m8, m8, m8], axis=0)
                if ii == 8 or ii == 0:
                    pf = jnp.exp2(sf - m)
                    if i0 == 0:
                        A[j][0] = _pack32(jnp.where(tri, pf, 0.0))
                        A[j][8] = _pack32(jnp.where(tri, 0.0, pf))
                    else:
                        A[j][8] = _pack32(pf)
                else:
                    ib = max(i0, 1)
                    A[j][ii] = _pack32(jnp.exp2(sm[32 * (ii - ib):32 * (ii - ib) + 32] - m))

            B = [[], [], [], []]
            for t in range(tmin, 12):
                dep = None
                if chain is not None and len(B[3]) >= chain[0]:
                    dep = B[chain[1]][-chain[0]][8:16] >> 31
                for j in range(4):
                    if t - j >= 0:
                        make(j, t - j, dep)
                a = [A[j][t - j] if 0 <= t - j <= 8 else None for j in range(4)]
                d0 = sel(m_even, a[0], a[1])
                d1 = sel(m_even, a[1], a[0])
                d2 = sel(m_even, a[2], a[3])
                d3 = sel(m_even, a[3], a[2])
                B[0].append(sel(m_lo, d0, d2))
                B[2].append(sel(m_lo, d2, d0))
                B[1].append(sel(m_mid, d1, d3))
                B[3].append(sel(m_mid, d3, d1))
            kb0 = tmin // 4
            vbase = qb + b - 2
            sub8w = lax.broadcasted_iota(jnp.int32, (8, 128 * (3 - kb0)), 0)
            outs = []
            for hh in range(4):
                pT = _b16(jnp.concatenate(B[hh], axis=0))
                r0 = 40 * g + 8 * hh
                va = jnp.concatenate([vt[vbase + ii, r0:r0 + 8, :] for ii in range(kb0, 3)], axis=1)
                vb = jnp.concatenate([vt[vbase + ii, r0 + 8:r0 + 16, :] for ii in range(kb0, 3)], axis=1)
                if hh < 2:
                    vb = jnp.where(sub8w >= 4, u32(ONE2), vb)
                else:
                    va = jnp.where(sub8w < 4, u32(ONE2), va)
                vw = _b16(jnp.concatenate([va, vb], axis=0))
                o = jnp.dot(vw, pT, preferred_element_type=f32)
                if hh < 2:
                    den = o[24:32]
                    val = o[0:24]
                else:
                    den = o[0:8]
                    val = o[8:32]
                inv = 1.0 / den
                val = val * jnp.concatenate([inv, inv, inv], axis=0)
                if hh:
                    val = pltpu.roll(val, 128 - 32 * hh, 1)
                outs.append(val)
            v2 = jnp.where(sub8 < 4, outs[0][16:24], outs[1][0:8])
            v7 = jnp.where(sub8 < 4, outs[2][16:24], outs[3][0:8])
            return jnp.concatenate([outs[0][0:16], v2, outs[1][8:24], outs[2][0:16], v7, outs[3][8:24]], axis=0)

        items = [(b, g) for b in range(nqb) for g in range(NG)]
        og = {}
        prev = None
        for n, it in enumerate(items):
            rs = []
            for ch in patterns[n % len(patterns)]:
                if ch == 'F':
                    run_fill(pieces, 1, keep + post + 1)
                elif ch == 'P':
                    if prev is not None:
                        og[prev[0]] = pv(prev[0][0], prev[0][1], prev[1])
                elif ch == 'a':
                    rs += qk(it[0], it[1], (0, 1))
                elif ch == 'b':
                    rs += qk(it[0], it[1], (2, 3))
                else:
                    rs += qk(it[0], it[1], (int(ch),))
            prev = (it, rs)
        run_fill(pieces, len(pieces), keep + post)
        og[prev[0]] = pv(prev[0][0], prev[0][1], prev[1])
        run_fill(pieces, len(pieces), keep)
        return jnp.concatenate([jnp.concatenate([og[(b, g)] for g in range(NG)], axis=0) for b in range(nqb)], axis=1)

    def wo_pieces(qb, lb, nqb, ot, ln):
        st = {'h': []}

        def xpose():
            if 'o' not in st:
                st['o'] = ot.T.astype(bf16)

        def part(n):
            xpose()
            st['h'].append(x_v[_ds(qb * QB, nqb * QB, QB), 128 * n:128 * n + 128].astype(f32)
                           + jnp.dot(st['o'], wo_v[:, 128 * n:128 * n + 128], preferred_element_type=f32))

        def get_hn():
            if 'hn' not in st:
                st['hn'] = _u32(ln(jnp.concatenate(st['h'], axis=1)).astype(bf16))
            return st['hn']

        def store():
            h_scr[_ds(lb * QB, nqb * QB, QB), :] = jnp.concatenate(st['h'], axis=1)
            hn_scr[_ds(lb * 64, nqb * 64, 64), :] = get_hn()

        return [P(part, n) for n in range(5)], get_hn, store, xpose

    def attn_block(qb, lb, nqb, pieces, patterns, keep, chain, post, ln, mid=None):
        pieces = list(pieces)
        ot = attention(qb, lb, nqb, pieces, patterns, keep, chain, post)
        wo, get_hn, store, _ = wo_pieces(qb, lb, nqb, ot, ln)
        for p in wo:
            p()
        run_fill(pieces, len(pieces), 0)
        store()
        if mid is not None:
            mid()
        for p in ffn_first(get_hn, lb, nqb):
            p()

    def prologue():
        cp_c1 = qcols(0, 128 * C1, 0)
        cp_c2 = qcols(128 * C1, 128 * (C1 + C2), 1)
        cp_c3 = qcols(128 * (C1 + C2), 3 * D, 2)
        cp_m = [wcopy(wo_hbm, wo_v, 3), wcopy(w1_hbm.at[0:FA, :], w1_v.at[0:FA, :], 3),
                wcopy(w3_hbm.at[0:FA, :], w3_v.at[0:FA, :], 3)]
        cp_r = [wcopy(w1_hbm.at[FA:F, :], w1_v.at[FA:F, :], 4), wcopy(w3_hbm.at[FA:F, :], w3_v.at[FA:F, :], 4),
                wcopy(w2_hbm, w2_v, 4), xcopy(2, 1, 4)]
        cp_x0 = xcopy(0, 1, 5)
        cp_x1 = xcopy(1, 1, 6)
        for c in [cp_x0, cp_x1, cp_c1, cp_c2, cp_c3] + cp_m + cp_r:
            c.start()

        k0, q0, v0, store0, ln0 = qkv_pieces(0, False)
        k1, q1, v1, store1, ln1 = qkv_pieces(1, False)
        qk0 = q0 + k0
        qk1 = q1 + k1
        cp_x0.wait()
        ln0()
        cp_x1.wait()
        ln1()
        cp_c1.wait()
        for n in range(C1):
            qk0[n]()
            qk1[n]()
        cp_c2.wait()
        for n in range(C1, C1 + C2):
            qk0[n]()
            qk1[n]()
        cp_c3.wait()
        for p in qk0[C1 + C2:]:
            p()
        wvt_v[...] = _u32(wqkv_v[:, 2 * D:3 * D].astype(f32).T.astype(bf16))
        for p in v0:
            p()
        store0()
        fill = qk1[C1 + C2:] + v1
        ot0 = attention(0, 0, 1, fill, PAT_QB0, 1, None, 2)
        wo0, get_hn0, st0, xp0 = wo_pieces(0, 0, 1, ot0, _ln)
        xp0()
        store1('kv')
        for c in cp_m:
            c.wait()
        fill = wo0 + fill + ffn_first(get_hn0, 0, 1)
        run_fill(fill, 2, 0)
        ot1 = attention(1, 1, 1, fill, PAT_QB1, 3, (6, 0), 2)
        st0()
        wo1, get_hn1, st1, _ = wo_pieces(1, 1, 1, ot1, _ln)
        for p in wo1:
            p()
        run_fill(fill, len(fill), 0)
        st1()
        store1('qv')
        for p in ffn_first(get_hn1, 1, 1):
            p()
        for c in cp_r:
            c.wait()
        xcopy(3, NSTEP - 3, 0).start()

    def steady(i):
        @pl.when(i == 2)
        def _():
            xcopy(3, NSTEP - 3, 0).wait()

        gu, w2, opening = ffn_rest((i - 1) * NB, 0, NB, False, 1, 7)
        kp, qp, vp, store, _ = qkv_pieces(i + 1, True)
        for p in opening:
            p()
        kinds = {'g': gu, 'k': kp, 'q': qp, 'v': vp, 'w': w2}
        fill = [kinds[c].pop(0) for c in FILL_STEADY]
        assert not any(kinds.values())
        attn_block(i * NB, 0, NB, fill, PAT_STEADY, 2, (4, 3), 1, _ln, store)

    def last(b):
        gu, w2, _ = ffn_rest((NSTEP - 2) * NB + b, b, 1, False, 0, 8)
        attn_block((NSTEP - 1) * NB + b, b, 1, gu + w2, PAT_LAST, 3, (5, 0), 2, P(_ln_chained, rows=32, dist=2))
        gu, w2, _ = ffn_rest((NSTEP - 1) * NB + b, b, 1, True, 0, 7)
        for p in gu + w2:
            p()

    def step(i, carry):
        @pl.when(i == 0)
        def _():
            prologue()

        @pl.when((i > 0) & (i < NSTEP - 1))
        def _():
            steady(i)

        @pl.when(i >= NSTEP - 1)
        def _():
            last(i - (NSTEP - 1))
        return carry

    lax.fori_loop(0, NSTEP - 1 + NB, step, 0)

    for i in range(NSTEP - 2):
        ocopy(i * NB, NB).wait()
    for b in range(NB):
        ocopy((NSTEP - 2) * NB + b, 1).wait()
    for n in (3, 4):
        for b in range(NB):
            ocopy_col((NSTEP - 1) * NB + b, 1, n).wait()


@jax.jit
def pallas_sequential_preLN__sliding_block__glu_gated_swiglu__prompt_kernel(A_x, A_wqkv, A_wo, B_x, B_w1, B_w3, B_w2):
    del B_x
    any_spec = pl.BlockSpec(memory_space=pl.ANY)
    return pl.pallas_call(
        _kernel,
        in_specs=[any_spec] * 6,
        out_specs=any_spec,
        out_shape=jax.ShapeDtypeStruct((1, S, D), bf16),
        scratch_shapes=[
            pltpu.VMEM((S, D), bf16),
            pltpu.VMEM((S, D), bf16),
            pltpu.VMEM((D, 3 * D), bf16),
            pltpu.VMEM((D, D), bf16),
            pltpu.VMEM((F, D), bf16),
            pltpu.VMEM((F, D), bf16),
            pltpu.VMEM((F, D), bf16),
            pltpu.VMEM((D // 2, D), u32),
            pltpu.VMEM((NG, S // 2, 128), u32),
            pltpu.VMEM((S // 128, D // 2, 128), u32),
            pltpu.VMEM((NG, T // 2, 128), u32),
            pltpu.VMEM((T, D), f32),
            pltpu.VMEM((T // 2, D), u32),
            pltpu.VMEM((T // 2, FA), u32),
            pltpu.SemaphoreType.DMA((7,)),
            pltpu.SemaphoreType.DMA((1,)),
        ],
        compiler_params=pltpu.CompilerParams(vmem_limit_bytes=100 * 1024 * 1024),
    )(A_x, A_wqkv, A_wo, B_w1.T, B_w3.T, B_w2)
```
